```python
import os as _os
_os.environ.setdefault('JAX_PLATFORMS', 'cpu')
import jax
import jax.numpy as jnp

def _softmax(x, axis=-1):
    return jax.nn.softmax(x, axis=axis)

def _gelu(x):
    return jax.nn.gelu(x, approximate=True)

def _silu(x):
    return jax.nn.silu(x)

def _sigmoid(x):
    return jax.nn.sigmoid(x)

def _layernorm(x, axis=-1, eps=1e-05):
    m = jnp.mean(x, axis=axis, keepdims=True)
    v = jnp.var(x, axis=axis, keepdims=True)
    return (x - m) / jnp.sqrt(v + eps)

def _scatter_add(tgt, idx, src, axis=0):
    return tgt.at[idx].add(src)

def _segment_sum(src, seg, n):
    return jax.ops.segment_sum(src, seg, n)

class _Rng:

    def __init__(self, key):
        self._k = key

    def _next(self):
        self._k, sub = jax.random.split(self._k)
        return sub

    def normal(self, shape):
        return jax.random.normal(self._next(), shape, dtype=jnp.bfloat16)

    def randint(self, lo, hi, shape):
        return jax.random.randint(self._next(), shape, lo, hi, dtype=jnp.int32)

    def uniform(self, shape, lo=0.0, hi=1.0):
        return jax.random.uniform(self._next(), shape, jnp.bfloat16, lo, hi)

    def permutation(self, n):
        return jax.random.permutation(self._next(), n)
kernel_name = 'interleave_layers__ssm_conv_h3__mixer_gmlp__prompt'

def setup_inputs():
    _rng = _Rng(jax.random.key(int.from_bytes(__import__("os").urandom(4), "little")))
    _w = lambda a: (lambda t: t.astype(jnp.bfloat16) if jnp.issubdtype(t.dtype, jnp.floating) else t)(jnp.asarray(a))

    def _A_setup():
        B, S, D = (1, 2048, 1024)
        ks = 4
        return {'q': _w((lambda *s: _rng.normal(s) * 0.05)(B, S, D)), 'k': _w((lambda *s: _rng.normal(s) * 1.6)(B, S, D)), 'v': _w((lambda *s: _rng.normal(s) * 1.6)(B, S, D)), 'shift_k': _w((lambda *s: _rng.normal(s) * 1.6)(D, ks) * 0.5), 'ssm_k': _w((lambda *s: _rng.normal(s) * 1.6)(D, S) * (1.0 / S ** 0.5)), 'ssm_D': _w((lambda *s: _rng.normal(s) * 1.6)(D))}
    _A_in = _A_setup()

    def _B_setup():
        B, S, D, F = (1, 2048, 1024, 3584)
        Fh = F // 2
        return {'x': _w((lambda *s: _rng.normal(s) * 0.05)(B, S, D)), 'w_in': _w((lambda *s: _rng.normal(s) * 0.8)(D, 2 * Fh)), 'w_sp': _w(0.01 * (lambda *s: _rng.normal(s) * 0.8)(S, S)), 'b_sp': _w(1.0 + 0.01 * (lambda *s: _rng.normal(s) * 0.2)(S)), 'w_out': _w((lambda *s: _rng.normal(s) * 0.2)(Fh, D))}
    _B_in = _B_setup()
    return {'A_q': _A_in['q'], 'A_k': _A_in['k'], 'A_v': _A_in['v'], 'A_shift_k': _A_in['shift_k'], 'A_ssm_k': _A_in['ssm_k'], 'A_ssm_D': _A_in['ssm_D'], 'B_x': _B_in['x'], 'B_w_in': _B_in['w_in'], 'B_w_sp': _B_in['w_sp'], 'B_b_sp': _B_in['b_sp'], 'B_w_out': _B_in['w_out']}

def reference(A_q, A_k, A_v, A_shift_k, A_ssm_k, A_ssm_D, B_x, B_w_in, B_w_sp, B_b_sp, B_w_out):

    def _A_ref(q, k, v, shift_k, ssm_k, ssm_D):
        B, S, D = q.shape
        ks = shift_k.shape[-1]
        k_pad = jnp.pad(k, ((0, 0), (ks - 1, 0), (0, 0)))
        k_shift = jnp.zeros_like(k)
        for t in range(ks):
            k_shift = k_shift + k_pad[:, t:t + S, :] * shift_k[:, ks - 1 - t][None, None, :]
        kv = k_shift * v
        L = 2 * S
        kv_pad = jnp.pad(kv, ((0, 0), (0, S), (0, 0)))
        kf_pad = jnp.pad(ssm_k, ((0, 0), (0, S)))
        kv_f = (lambda x, axes=(-2, -1): jnp.fft.rfft2(x.astype(jnp.float32), axes=axes))(kv_pad[:, None, :, :], axes=(1, 2))
        kf_f = (lambda x, axes=(-2, -1): jnp.fft.rfft2(x.astype(jnp.float32), axes=axes))(kf_pad[:, None, :], axes=(1, 2))
        kf_f = (lambda x, *d: x.transpose(*d))(kf_f, 1, 2, 0)
        y_f = kv_f * kf_f[None, :, :, :]
        y = (lambda x, s, axes=(-2, -1): jnp.fft.irfft2(x, s=s, axes=axes).astype(jnp.bfloat16))(y_f, (1, L), axes=(1, 2))[:, 0, :S, :]
        y = y + kv * ssm_D[None, None, :]
        return q * y

    def _B_ref(x, w_in, w_sp, b_sp, w_out):
        B, S, D = x.shape
        F = w_in.shape[-1]
        Fh = F // 2
        z = _gelu(jnp.einsum('bsd,df->bsf', x, w_in))
        z1 = z[..., :Fh].copy()
        z2 = _layernorm(z[..., Fh:], axis=-1)
        g = jnp.einsum('ts,bsf->btf', w_sp, z2) + b_sp[None, :, None]
        return jnp.einsum('bsf,fd->bsd', z1 * g, w_out)
    x = A_q
    x = x + _A_ref(_layernorm(x, axis=-1), A_k, A_v, A_shift_k, A_ssm_k, A_ssm_D)
    x = x + _B_ref(_layernorm(x, axis=-1), B_w_in, B_w_sp, B_b_sp, B_w_out)
    x = x + _A_ref(_layernorm(x, axis=-1), A_k, A_v, A_shift_k, A_ssm_k, A_ssm_D)
    x = x + _B_ref(_layernorm(x, axis=-1), B_w_in, B_w_sp, B_b_sp, B_w_out)
    return x
```

```python
import functools
import numpy as np
import jax
import jax.numpy as jnp
import jax.experimental.pallas as pl
import jax.experimental.pallas.tpu as pltpu

S, D, F = 2048, 1024, 3584
FH = F // 2
B = 128
NB = S // B
TM = 256
NT = S // TM
EPS = 1e-5
F32, BF16 = jnp.float32, jnp.bfloat16
CN = 256
NC = FH // CN
OXC, OXS, OHC, OHS = 0, D + 128, 2 * (D + 128), 3 * (D + 128)
WSP = 4 * D + 3 * 128


def _dft_mats():
    ks = np.concatenate([np.arange(0, B, 2), np.arange(1, B, 2)])
    th = np.pi * (2 * ks + 1) / (2 * B)
    n = np.arange(B)
    ang = th[:, None] * n[None, :]
    f = np.concatenate([np.cos(ang), np.sin(ang)], axis=0)
    g = f.T / B
    return f.astype(np.float32), g.astype(np.float32)


def _ln(x):
    m = jnp.mean(x, axis=-1, keepdims=True)
    xc = x - m
    v = jnp.mean(xc * xc, axis=-1, keepdims=True)
    return xc * jax.lax.rsqrt(v + EPS)


def _gelu(x):
    c = np.float32(np.sqrt(2.0 / np.pi))
    inner = x * (c + (c * np.float32(0.044715)) * (x * x))
    hx = 0.5 * x
    return hx + hx * jnp.tanh(inner)


def _dot(a, b):
    return jnp.dot(a, b, preferred_element_type=F32)


def kernel(q_hbm, k_hbm, v_hbm, shk_ref, sk_hbm, sd_ref, win_hbm, wsp_hbm, bsp_ref, wout_hbm,
           f_ref, g_ref, zero_v, out_hbm,
           win_v, wsp_v, wout_v, z1_v, z2a_v, x_v, y_v, h_v, q_v, bb_v,
           kv_v, sk_v, sp_v, ys_v,
           sem_in, sem_w, sem_out):
    k_v = kv_v.at[:, 0:D]
    v_v = kv_v.at[:, D:2 * D]
    z2b_v = kv_v.at[:, 0:FH]
    u_v = sk_v.at[0:2 * TM, 0:FH]

    HS = (slice(0, TM), slice(TM, 2 * TM))

    def a_layer(x, y, rows, hs):
        x1 = x + _ln(x) * y
        x_v[rows, :] = x1
        h_v[hs, :] = _ln(x1).astype(BF16)

    def mm1_steps(rows, hs, z2_dst):
        zs = []
        def z2_step(c):
            zs.append(_gelu(_dot(h_v[hs, :], win_v[:, FH + c * CN:FH + (c + 1) * CN])))
            if c == NC - 1:
                z2 = jnp.concatenate(zs, axis=1)
                z2_dst[rows, :] = _ln(z2).astype(BF16)
        def z1_step(c):
            z1_v[rows, c * CN:(c + 1) * CN] = _gelu(_dot(h_v[hs, :], win_v[:, c * CN:(c + 1) * CN]))
        return ([functools.partial(z2_step, c) for c in range(NC)]
                + [functools.partial(z1_step, c) for c in range(NC)])

    def mm1(rows, hs, z2_dst):
        for s in mm1_steps(rows, hs, z2_dst):
            s()

    w_copies = [pltpu.make_async_copy(win_hbm, win_v, sem_w.at[0]),
                pltpu.make_async_copy(wsp_hbm, wsp_v, sem_w.at[1]),
                pltpu.make_async_copy(wout_hbm, wout_v, sem_w.at[2])]

    def phase1():
        def in_copies(t):
            r = pl.ds(t * TM, TM)
            return [pltpu.make_async_copy(k_hbm.at[0, r], k_v.at[r], sem_in.at[t, 0]),
                    pltpu.make_async_copy(v_hbm.at[0, r], v_v.at[r], sem_in.at[t, 1]),
                    pltpu.make_async_copy(sk_hbm.at[:, r], sk_v.at[:, r], sem_in.at[t, 2]),
                    pltpu.make_async_copy(q_hbm.at[0, r], q_v.at[r], sem_in.at[t, 3])]
        for t in range(2):
            for c in in_copies(t):
                c.start()
        w_copies[0].start()
        for t in range(2, NT):
            for c in in_copies(t):
                c.start()
        w_copies[1].start()
        w_copies[2].start()

        eye = (jax.lax.broadcasted_iota(jnp.int32, (8, 4), 0)
               == jax.lax.broadcasted_iota(jnp.int32, (8, 4), 1)).astype(BF16)
        shk = jax.lax.dot_general(eye, shk_ref[...], (((1,), (1,)), ((), ())), preferred_element_type=F32)
        sd = sd_ref[...].astype(F32)
        bb_v[...] = jnp.transpose(jnp.broadcast_to(bsp_ref[...].astype(F32), (128, S)))

        st = {"hprev": None, "dep": (jnp.zeros((8, 128), F32), jnp.zeros((8, 128), F32))}

        def wait_in(t):
            for c in in_copies(t):
                c.wait()

        def fwd_x(m):
            r = slice(m * B, (m + 1) * B)
            kf = k_v[r, :].astype(F32)
            if m == 0:
                prev = jnp.zeros((8, D), F32)
            else:
                prev = k_v[m * B - 16:m * B, :].astype(F32)[8:16]
            kx = jnp.concatenate([prev, kf], axis=0)
            ksh = kf * shk[0:1]
            for j in range(1, 4):
                ksh = ksh + pltpu.roll(kx, j, axis=0)[8:] * shk[j:j + 1]
            kv = ksh * v_v[r, :].astype(F32)
            y_v[r, :] = kv * sd
            xf = _dot(f_ref[...], kv.astype(BF16))
            sp_v[m, :, OXC:OXC + D] = xf[0:B]
            sp_v[m, :, OXS:OXS + D] = xf[B:2 * B]

        def fwd_h(m):
            r = slice(m * B, (m + 1) * B)
            hraw = jax.lax.dot_general(f_ref[...], sk_v[:, r], (((1,), (1,)), ((), ())), preferred_element_type=F32)
            hprev = st["hprev"]
            hb = B // 2
            if hprev is None:
                sp_v[m, :, OHC:OHC + D] = hraw[0:B]
                sp_v[m, :, OHS:OHS + D] = hraw[B:2 * B]
            else:
                sp_v[m, 0:hb, OHC:OHC + D] = hraw[0:hb] + hprev[B:B + hb]
                sp_v[m, hb:B, OHC:OHC + D] = hraw[hb:B] - hprev[B + hb:2 * B]
                sp_v[m, 0:hb, OHS:OHS + D] = hraw[B:B + hb] - hprev[0:hb]
                sp_v[m, hb:B, OHS:OHS + D] = hraw[B + hb:2 * B] + hprev[hb:B]
            st["hprev"] = hraw

        def chain(m):
            slot = m % 4
            nr = B // 8
            def body(p, carry):
                dr, di = carry
                r0 = pl.multiple_of((p % nr) * 8, 8)
                c0 = pl.multiple_of((p // nr) * 128, 128)
                zm = zero_v[...]
                yr = pltpu.bitcast(pltpu.bitcast(dr, jnp.int32) & zm, F32)
                yi = pltpu.bitcast(pltpu.bitcast(di, jnp.int32) & zm, F32)
                for i in range(m + 1):
                    xr = sp_v[i, pl.ds(r0, 8), pl.ds(OXC + c0, 128)]
                    xi = sp_v[i, pl.ds(r0, 8), pl.ds(OXS + c0, 128)]
                    hr = sp_v[m - i, pl.ds(r0, 8), pl.ds(OHC + c0, 128)]
                    hi = sp_v[m - i, pl.ds(r0, 8), pl.ds(OHS + c0, 128)]
                    yr = (yr + xr * hr) - xi * hi
                    yi = (yi + xr * hi) + xi * hr
                ys_v[slot, pl.ds(r0, 8), pl.ds(c0, 128)] = yr
                ys_v[slot, pl.ds(B + r0, 8), pl.ds(c0, 128)] = yi
                return yr, yi
            st["dep"] = jax.lax.fori_loop(0, nr * (D // 128), body, st["dep"], unroll=True)

        def wide(m):
            slot = m % 4
            for c0 in range(0, D, 512):
                for r0 in range(0, B, 8):
                    yr = yi = None
                    for i in range(m + 1):
                        xr = sp_v[i, r0:r0 + 8, OXC + c0:OXC + c0 + 512]
                        xi = sp_v[i, r0:r0 + 8, OXS + c0:OXS + c0 + 512]
                        hr = sp_v[m - i, r0:r0 + 8, OHC + c0:OHC + c0 + 512]
                        hi = sp_v[m - i, r0:r0 + 8, OHS + c0:OHS + c0 + 512]
                        tr = xr * hr - xi * hi
                        ti = xr * hi + xi * hr
                        yr = tr if yr is None else yr + tr
                        yi = ti if yi is None else yi + ti
                    ys_v[slot, r0:r0 + 8, c0:c0 + 512] = yr
                    ys_v[slot, B + r0:B + r0 + 8, c0:c0 + 512] = yi

        def inv_a(t):
            ys = []
            for m in (2 * t, 2 * t + 1):
                r = slice(m * B, (m + 1) * B)
                y = y_v[r, :] + _dot(g_ref[...], ys_v[m % 4].astype(BF16))
                y_v[r, :] = y
                ys.append(y)
            rows = slice(t * TM, (t + 1) * TM)
            a_layer(q_v[rows, :].astype(F32), jnp.concatenate(ys, axis=0), rows, HS[t % 2])

        def fwd_steps(t):
            return [functools.partial(fn, m) for m in (2 * t, 2 * t + 1) for fn in (fwd_h, fwd_x)]

        wait_in(0)
        for s in fwd_steps(0):
            s()
        wide(0)
        wide(1)
        inv_a(0)
        wait_in(1)
        for s in fwd_steps(1):
            s()
        chain(2)
        chain(3)
        w_copies[0].wait()
        for t in range(NT):
            rows = slice(t * TM, (t + 1) * TM)
            steps = mm1_steps(rows, HS[t % 2], z2a_v)
            extra = {}
            if t + 2 < NT:
                fs = fwd_steps(t + 2)
                extra.setdefault(0, []).append(functools.partial(wait_in, t + 2))
                for n, s in enumerate(fs):
                    extra.setdefault(1 + n, []).append(s)
                extra.setdefault(INV_AT + 1, []).append(functools.partial(chain, 2 * t + 4))
                extra.setdefault(INV_AT + 1, []).append(functools.partial(chain, 2 * t + 5))
            if t + 1 < NT:
                extra.setdefault(INV_AT, []).append(functools.partial(inv_a, t + 1))
            for n, s in enumerate(steps):
                for e in extra.get(n, []):
                    e()
                s()

    INV_AT = 11
    phase1()

    def phase23():
        def mm2(rows, hs, z2_src):
            bb = bb_v[rows, :]
            bb = jnp.concatenate([bb] * (CN // 128), axis=1)
            for c in range(NC):
                cs = slice(c * CN, (c + 1) * CN)
                g = _dot(wsp_v[rows, :], z2_src[:, cs]) + bb
                u_v[hs, cs] = (z1_v[rows, cs] * g).astype(BF16)

        def mm3(rows, hs):
            return x_v[rows, :] + _dot(u_v[hs, :], wout_v[...])

        def rows2(i):
            r0 = pl.multiple_of(i * (2 * TM), 2 * TM)
            return pl.ds(r0, TM), pl.ds(r0 + TM, TM)

        w_copies[1].wait()
        w_copies[2].wait()
        def p2(i, _):
            ra, rb = rows2(i)
            mm2(ra, HS[0], z2a_v)
            mm2(rb, HS[1], z2a_v)
            a_layer(mm3(ra, HS[0]), y_v[ra, :], ra, HS[0])
            a_layer(mm3(rb, HS[1]), y_v[rb, :], rb, HS[1])
            mm1(ra, HS[0], z2b_v)
            mm1(rb, HS[1], z2b_v)
            return 0
        jax.lax.fori_loop(0, NT // 2, p2, 0)

        o_v = q_v
        def out_copy(i):
            r = pl.ds(pl.multiple_of(i * (2 * TM), 2 * TM), 2 * TM)
            return pltpu.make_async_copy(o_v.at[r], out_hbm.at[0, r], sem_out.at[i])
        def p3(i, _):
            ra, rb = rows2(i)
            mm2(ra, HS[0], z2b_v)
            mm2(rb, HS[1], z2b_v)
            o_v[ra, :] = mm3(ra, HS[0]).astype(BF16)
            o_v[rb, :] = mm3(rb, HS[1]).astype(BF16)
            out_copy(i).start()
            return 0
        jax.lax.fori_loop(0, NT // 2, p3, 0)
        for i in range(NT // 2):
            out_copy(i).wait()

    phase23()


@jax.jit
def pallas_interleave_layers__ssm_conv_h3__mixer_gmlp__prompt_kernel(A_q, A_k, A_v, A_shift_k, A_ssm_k, A_ssm_D, B_x, B_w_in, B_w_sp, B_b_sp, B_w_out):
    f, g = _dft_mats()
    any_ = pl.BlockSpec(memory_space=pl.ANY)
    vm = pl.BlockSpec(memory_space=pltpu.VMEM)
    return pl.pallas_call(
        kernel,
        out_shape=jax.ShapeDtypeStruct((1, S, D), BF16),
        in_specs=[any_, any_, any_, vm, any_, vm, any_, any_, vm, any_, vm, vm, vm],
        out_specs=any_,
        scratch_shapes=[
            pltpu.VMEM((D, F), BF16), pltpu.VMEM((S, S), BF16), pltpu.VMEM((FH, D), BF16),
            pltpu.VMEM((S, FH), F32), pltpu.VMEM((S, FH), BF16),
            pltpu.VMEM((S, D), F32), pltpu.VMEM((S, D), F32),
            pltpu.VMEM((2 * TM, D), BF16), pltpu.VMEM((S, D), BF16),
            pltpu.VMEM((S, 128), F32),
            pltpu.VMEM((S, 2 * D), BF16), pltpu.VMEM((D, S), BF16),
            pltpu.VMEM((NB, B, WSP), F32), pltpu.VMEM((4, 2 * B, D), F32),
            pltpu.SemaphoreType.DMA((NT, 4)), pltpu.SemaphoreType.DMA((3,)), pltpu.SemaphoreType.DMA((NT // 2,)),
        ],
        compiler_params=pltpu.CompilerParams(vmem_limit_bytes=127 * 1024 * 1024),
    )(A_q, A_k, A_v, A_shift_k, A_ssm_k, A_ssm_D.reshape(1, D), B_w_in, B_w_sp, B_b_sp.reshape(1, S), B_w_out,
      jnp.asarray(f, BF16), jnp.asarray(g, BF16), jnp.asarray(np.zeros((8, 128), np.int32)))
```

```python
import functools
import numpy as np
import jax
import jax.numpy as jnp
import jax.experimental.pallas as pl
import jax.experimental.pallas.tpu as pltpu

S, D, F = 2048, 1024, 3584
FH = F // 2
B = 128
NB = S // B
TM = 256
NT = S // TM
EPS = 1e-5
F32, BF16, I32 = jnp.float32, jnp.bfloat16, jnp.int32
CN = 256
NC = FH // CN
OXC, OXS, OHC, OHS = 0, D + 128, 2 * (D + 128), 3 * (D + 128)
WSP = 4 * D + 3 * 128
NYS = 6
P = functools.partial
SCOPES = False
ONLY = None
OPT = dict(frA=0, frB=0, split=50, b0=-700, R=16, xdyn=0, o=3, a0=1000, a1=1500, h0=520, h1=300, pr=0, W=128, fence=1)

ORD = {0: 's0 s1 s2 h0 h1 w600 x0 x1 s3 s4 w500 i s5 a s6 n',
       1: 's0 h0 s1 h1 s2 x0 s3 x1 s4 s5 s6 s7 i s8 e0 s9 s10 s11 s12 s13',
       2: 'e0 s0 h0 s1 h1 s2 x0 s3 x1 s4 s5 s6 s7 i s8 s9 s10 s11 s12 s13',
       4: 'e0 s0 h0 s1 h1 s2 x0 s3 x1 s4 s5 s6 s7 i s8 e1 s9 s10 s11 s12 s13',
       7: 's0 s1 s2 s3 s4 s5 s6 s7 s8 s9 s10 s11 s12 s13'}

TICK, MARGIN, LATE, ENDM = 112, 300, 700, 400
SG, LND, KVD, HD = 330, 3, 3, 2


def _dft_mats():
    ks = np.concatenate([np.arange(0, B, 2), np.arange(1, B, 2)])
    th = np.pi * (2 * ks + 1) / (2 * B)
    n = np.arange(B)
    ang = th[:, None] * n[None, :]
    f = np.concatenate([np.cos(ang), np.sin(ang)], axis=0)
    g = np.empty((B, 2 * B))
    g[:, 0::2] = np.cos(ang).T / B
    g[:, 1::2] = np.sin(ang).T / B
    return f.astype(np.float32), g.astype(np.float32)


def _plan():
    done = {(0, 0), (1, 0), (1, 1)}
    plan = {}
    def take(key, pairs):
        jobs = {}
        for m, i in pairs:
            done.add((m, i))
            jobs.setdefault(m, []).append(i)
        plan[key] = sorted(jobs.items())
    quota = {0: 6, 1: 14, 2: 18, 3: 18, 4: 17, 5: 17}
    pend = []
    for t in range(NT - 1):
        take((t, 'A'), pend)
        take((t, 'H'), [(m, i) for m in (2 * t + 2, 2 * t + 3) for i in range(m + 1) if (m, i) not in done])
        a = 2 * t + 3
        cand = [(m, i) for m in range(2 * t + 4, min(2 * t + 4 + NYS, NB)) for i in range(m + 1)
                if i <= a and m - i <= a and (m, i) not in done][:quota.get(t, 0)]
        tgt = int(round(0.01 * OPT['split'] * len(cand))) if t else 0
        cuts = [n for n in range(len(cand) + 1) if n in (0, len(cand)) or cand[n][0] != cand[n - 1][0]]
        nb = min(cuts, key=lambda n: abs(n - tgt))
        if abs(nb - tgt) > 2:
            nb = tgt
        take((t, 'B'), cand[:nb])
        pend = cand[nb:]
        for c in pend:
            done.add(c)
    assert len(done) == NB * (NB + 1) // 2
    return plan


def _ln(x):
    m = jnp.mean(x, axis=-1, keepdims=True)
    xc = x - m
    v = jnp.mean(xc * xc, axis=-1, keepdims=True)
    return xc * jax.lax.rsqrt(v + EPS)


def _ln2(x):
    m = jnp.mean(x, axis=-1, keepdims=True)
    xc = x - m
    v = jnp.mean(xc * xc, axis=-1, keepdims=True)
    return xc * (0.5 * jax.lax.rsqrt(v + 4 * EPS))


def _gelu(x):
    c = np.float32(np.sqrt(2.0 / np.pi))
    inner = x * (c + (c * np.float32(0.044715)) * (x * x))
    return x + x * jnp.tanh(inner)


def _dot(a, b):
    return jnp.dot(a, b, preferred_element_type=F32)


class _NoScope:
    def __enter__(self): return self
    def __exit__(self, *a): return False


def _scope(name):
    return jax.named_scope(name) if SCOPES else _NoScope()


def kernel(q_hbm, k_hbm, v_hbm, shk_hbm, sk_hbm, sd_hbm, win_hbm, wsp_hbm, bsp_hbm, wout_hbm,
           f_hbm, g_hbm, zs_hbm, out_hbm,
           win_v, wsp_v, wout_v, z1_v, z2a_v, x_v3, y_v3, h_v, q_v3, bb_v,
           kv_v, sk_v, zt_v, shk_v, clk_v, shk_ref, sd_ref, bsp_ref, f_ref, g_ref, zs_ref,
           sem_in, sem_w, sem_s, sem_out, *bufs):
    sps, yss = bufs[:NT], bufs[NT:]
    x_v, y_v, q_v = x_v3.at[0], y_v3.at[0], q_v3.at[0]
    k_v = kv_v.at[:, 0:D]
    v_v = kv_v.at[:, D:2 * D]
    z2b_v = kv_v.at[:, 0:FH]
    u_v = sk_v.at[0:2 * TM, 0:FH]
    HS = (slice(0, TM), slice(TM, 2 * TM), slice(2 * TM, 3 * TM))

    bi = lambda x: pltpu.bitcast(x, I32)
    hi = lambda w: pltpu.bitcast(w & np.int32(-65536), F32)
    lo = lambda w: pltpu.bitcast(w << 16, F32)
    pk = lambda a, b: bi(pltpu.pack_elementwise([a, b], packed_dtype=BF16))
    bc = lambda m: jnp.broadcast_to(m, (m.shape[0], 128))
    wide = lambda m, n: jnp.concatenate([m] * n, axis=1)
    rows8 = lambda x: [x[r:r + 8, c:c + 128] for r in range(0, x.shape[0], 8) for c in range(0, x.shape[1], 128)]
    cols = lambda x: [x[:, c:c + 128] for c in range(0, x.shape[1], 128)]

    WG = ((FH, FH + 3 * CN), (FH + 3 * CN, FH + 5 * CN), (FH + 5 * CN, F), (0, 3 * CN), (3 * CN, FH))
    wc = [pltpu.make_async_copy(win_hbm.at[:, a:b], win_v.at[:, a:b], sem_w.at[n]) for n, (a, b) in enumerate(WG)]
    def wsp_copy(n):
        r = pl.ds(pl.multiple_of(n * TM, TM), TM)
        return pltpu.make_async_copy(wsp_hbm.at[r], wsp_v.at[r], sem_w.at[7 + n])
    wout_copies = [pltpu.make_async_copy(wout_hbm.at[n * (FH // 2):(n + 1) * (FH // 2)],
                                         wout_v.at[n * (FH // 2):(n + 1) * (FH // 2)], sem_w.at[5 + n]) for n in range(2)]
    small = [pltpu.make_async_copy(a, b, sem_s.at[n]) for n, (a, b) in enumerate(
        [(zs_hbm, zs_ref), (f_hbm, f_ref), (shk_hbm, shk_ref), (sd_hbm, sd_ref), (bsp_hbm, bsp_ref), (g_hbm, g_ref)])]

    def tile_copies(t):
        r = pl.ds(t * TM, TM)
        return [pltpu.make_async_copy(k_hbm.at[0, r], k_v.at[r], sem_in.at[t, 0]),
                pltpu.make_async_copy(v_hbm.at[0, r], v_v.at[r], sem_in.at[t, 1]),
                pltpu.make_async_copy(sk_hbm.at[:, r], sk_v.at[:, r], sem_in.at[t, 2]),
                pltpu.make_async_copy(q_hbm.at[0, r], q_v.at[r], sem_in.at[t, 3])]
    inc = [tile_copies(t) for t in range(NT)]

    def start(cs):
        for c in cs:
            c.start()

    def wait(cs):
        for c in cs:
            c.wait()

    def a_layer(x, y, rows, hs):
        x1 = x + _ln(x) * y
        x_v[rows, :] = x1
        h_v[hs, :] = _ln(x1).astype(BF16)

    def mm1(rows, hs, z2_dst):
        zs = [_gelu(_dot(h_v[hs, :], win_v[:, FH + c * CN:FH + (c + 1) * CN])) for c in range(NC)]
        z2_dst[rows, :] = _ln2(jnp.concatenate(zs, axis=1)).astype(BF16)
        for c in range(NC):
            z1_v[rows, c * CN:(c + 1) * CN] = _gelu(_dot(h_v[hs, :], win_v[:, c * CN:(c + 1) * CN]))

    def mm2(rows, hs, z2_src, act=False):
        bb = wide(bb_v[rows, :], CN // 128)
        for c in range(NC):
            cs = slice(c * CN, (c + 1) * CN)
            g = _dot(wsp_v[rows, :], z2_src[:, cs]) + bb
            z1 = z1_v[rows, cs]
            u_v[hs, cs] = ((_gelu(z1) if act else z1) * g).astype(BF16)

    def mm3(rows, hs):
        return x_v[rows, :] + _dot(u_v[hs, :], wout_v[...])

    with _scope("pro_init"):
        first = small[0:5] + inc[0][2:3]
        start(first)
        for sm, grp in zip(first, (inc[0][0:2] + small[5:], [inc[0][3], wc[0]], inc[1][0:3], [wc[1]], [inc[1][3]],
                                   [wc[2]])):
            sm.wait()
            start(grp)
    z0 = zs_ref[0]
    dyn = (z0, z0 + 1)
    dz = [z0 * k for k in range(4)]
    zm = jnp.full((8, 128), z0, I32)
    with _scope("pro_bb"):
        shk_v[...] = shk_ref[...].astype(F32)
        bb_v[...] = jnp.transpose(jnp.broadcast_to(0.5 * bsp_ref[...].astype(F32).reshape(1, S), (128, S)))

    st = {"hprev": None, "clk": jax.lax.broadcasted_iota(I32, (8, 128), 1) & zm, "fresh": ()}
    qs = {}
    started = set()

    def lnk(h):
        h00 = pltpu.bitcast(bi(h[0:16, 0:128]) | st["clk"], BF16)
        return jnp.concatenate([jnp.concatenate([h00, h[0:16, 128:]], axis=1), h[16:]], axis=0)

    def lhs(hs):
        return lnk(h_v[hs, :])

    def rs(base, off, n):
        if isinstance(base, int):
            return slice(base + off, base + off + n)
        return pl.ds(pl.multiple_of(base + off, n), n)

    def z2_step(hs, zr, c):
        zt_v[0, zr, c * CN:(c + 1) * CN] = _gelu(_dot(lhs(hs), win_v[:, FH + c * CN:FH + (c + 1) * CN]))

    def z1_step(hs, rows, act, c):
        z = _dot(lhs(hs), win_v[:, c * CN:(c + 1) * CN])
        z1_v[rows, c * CN:(c + 1) * CN] = _gelu(z) if act else z

    def g_step(rows, us, c):
        cs = slice(c * CN, (c + 1) * CN)
        g = _dot(lnk(wsp_v[rows, :]), z2a_v[:, cs]) + wide(bb_v[rows, :], CN // 128)
        u_v[us, cs] = (_gelu(z1_v[rows, cs]) * g).astype(BF16)

    def o_step(rows, us, xt, link, c):
        cs = slice(c * CN, (c + 1) * CN)
        u = u_v[us, :]
        xt[0, 0:u.shape[0], cs] = x_v[rows, cs] + _dot(lnk(u) if link else u, wout_v[:, cs])

    def ssum(xs):
        s_ = xs[0]
        for v in xs[1:]:
            s_ = s_ + v
        return jnp.sum(s_, axis=-1, keepdims=True) * (1.0 / (128 * len(xs)))

    def st_mean(key, x):
        m = qs[key] = bc(ssum(cols(x)))
        return [bi(m)]

    def st_rstd(key, mkey, x, half=False):
        m = qs[mkey]
        xc = [v - m for v in cols(x)]
        r = jax.lax.rsqrt(ssum([v * v for v in xc]) + (4 * EPS if half else EPS))
        r = qs[key] = bc(0.5 * r if half else r)
        return [bi(r)]

    def st_out(dst, r0, g, x, mkey, rkey):
        n = x.shape[1] // 128
        m = jnp.concatenate([pltpu.bitcast(bi(qs[mkey, 2 * g + j]) | st["clk"], F32) for j in range(2)], axis=0)
        r = jnp.concatenate([qs[rkey, 2 * g + j] for j in range(2)], axis=0)
        dst[rs(r0, 16 * g, 16), :] = ((x - wide(m, n)) * wide(r, n)).astype(BF16)
        return []

    def nrm_q(cx, g, stage):
        dst, base, z0r = cx
        if stage == 0:
            return st_mean(('nm', g), zt_v[dz[1], rs(z0r, 8 * g, 8), :])
        if stage == 1:
            return st_rstd(('nr', g), ('nm', g), zt_v[dz[2], rs(z0r, 8 * g, 8), :], True)
        return st_out(dst, base, g, zt_v[dz[3], rs(z0r, 16 * g, 16), :], 'nm', 'nr')

    def a_q(cx, g, stage):
        src, s0, base, xs, x0, h0 = cx
        r = rs(base, 8 * g, 8)
        if stage <= 2:
            x = src[dz[stage + 1], rs(s0, 8 * g, 8), :].astype(F32)
        if stage == 0:
            return st_mean(('am', g), x)
        if stage == 1:
            return st_rstd(('ar', g), ('am', g), x)
        if stage == 2:
            x1 = x + ((x - wide(qs['am', g], 8)) * wide(qs['ar', g], 8)) * y_v3[dz[1], r, :]
            x_v[r, :] = x1
            if xs is not x_v3:
                xs[0, rs(x0, 8 * g, 8), :] = x1
            return st_mean(('am', g), x1)
        if stage == 3:
            return st_rstd(('ar', g), ('am', g), xs[0, rs(x0, 8 * g, 8), :])
        return st_out(h_v, h0, g, xs[0, rs(x0, 16 * g, 16), :], 'am', 'ar')

    def kv_q(m, c):
        cs = slice(c * 128, (c + 1) * 128)
        if m == 0:
            kw = jnp.concatenate([jnp.zeros((8, 128), I32), bi(k_v[0:B, cs])], axis=0)
        else:
            kw = bi(k_v[m * B - 16:(m + 1) * B, cs])
        k0 = kw[8:]
        k1 = pltpu.roll(kw, 1, axis=0)[8:]
        k2 = pltpu.roll(kw, 2, axis=0)[8:]
        w = [jnp.broadcast_to(shk_v[j:j + 1, cs], (8, 128)) for j in range(4)]
        vw = bi(v_v[m * B:(m + 1) * B, cs])
        out = []
        for n in range(8):
            r = slice(8 * n, 8 * n + 8)
            e0, o0, e1, o1, o2 = lo(k0[r]), hi(k0[r]), lo(k1[r]), hi(k1[r]), hi(k2[r])
            w0 = w[0] if (not out or m < 2) else pltpu.bitcast(bi(w[0]) | (out[-1] & zm), F32)
            se = ((e0 * w0 + o1 * w[1]) + e1 * w[2]) + o2 * w[3]
            so = ((o0 * w0 + e0 * w[1]) + o1 * w[2]) + e1 * w[3]
            out.append(pk(se * lo(vw[r]), so * hi(vw[r])))
        qs['kv', m, c] = jnp.concatenate(out, axis=0)
        return [out[-1]]

    def fwd_x(m):
        kvb = pltpu.bitcast(jnp.concatenate([qs.pop(('kv', m, c)) for c in range(8)], axis=1), BF16)
        xf = _dot(f_ref[...], kvb)
        sps[m // 2][m % 2, 0:B, OXC:OXC + D] = xf[0:B]
        sps[m // 2][m % 2, 0:B, OXS:OXS + D] = xf[B:2 * B]
        if m % 2 and OPT['fence']:
            sps[m // 2][z0, 0:8, D:D + 128] = jnp.zeros((8, 128), F32)

    def fwd_h(m):
        hraw = jax.lax.dot_general(f_ref[...], sk_v[:, m * B:(m + 1) * B], (((1,), (1,)), ((), ())),
                                   preferred_element_type=F32)
        hprev = st["hprev"]
        hb = B // 2
        sp = sps[m // 2]
        if hprev is None:
            hraw = jnp.concatenate([hraw[0:B] + sd_ref[...].astype(F32).reshape(1, D), hraw[B:2 * B]], axis=0)
            sp[m % 2, 0:B, OHC:OHC + D] = hraw[0:B]
            sp[m % 2, 0:B, OHS:OHS + D] = hraw[B:2 * B]
        else:
            sp[m % 2, 0:hb, OHC:OHC + D] = hraw[0:hb] + hprev[B:B + hb]
            sp[m % 2, hb:B, OHC:OHC + D] = hraw[hb:B] - hprev[B + hb:2 * B]
            sp[m % 2, 0:hb, OHS:OHS + D] = hraw[B:B + hb] - hprev[0:hb]
            sp[m % 2, hb:B, OHS:OHS + D] = hraw[B + hb:2 * B] + hprev[hb:B]
        st["hprev"] = hraw

    def piece(m, iis, acc, final, R, W, p, fr=0):
        nr = B // R
        r0 = (p % nr) * R
        c0 = (p // nr) * W
        ys = yss[m % NYS]
        yr = yi = None
        if acc:
            yr = ys[0, r0:r0 + R, c0:c0 + W]
            yi = ys[0, B + r0:B + r0 + R, c0:c0 + W]
        def ld(b, off):
            j = dyn[b % 2] if b // 2 in st["fresh"] and not OPT['fence'] else b % 2
            return sps[b // 2][j, r0:r0 + R, off + c0:off + c0 + W]
        for i in iis:
            xr, xi, hr, hi_ = ld(i, OXC), ld(i, OXS), ld(m - i, OHC), ld(m - i, OHS)
            yr = (xr * hr if yr is None else yr + xr * hr) - xi * hi_
            yi = (xr * hi_ if yi is None else yi + xr * hi_) + xi * hr
        if final:
            r_ = qs['y', m, p] = pk(yr, yi)
            return rows8(r_)
        if fr:
            yr = pltpu.bitcast(bi(yr) | st["clk"], F32)
            yi = pltpu.bitcast(bi(yi) | st["clk"], F32)
        ys[0, r0:r0 + R, c0:c0 + W] = yr
        ys[0, B + r0:B + r0 + R, c0:c0 + W] = yi
        return rows8(bi(yr) | bi(yi)) if fr != 1 else []

    def pieces(jobs, final, R=None, W=None, interleave=False, fr=0):
        R = R or OPT['R']
        W = W or OPT['W']
        out = []
        for m, iis in jobs:
            out.append([P(piece, m, iis, m in started, final, R, W, p, fr) for p in range((B // R) * (D // W))])
            started.add(m)
        if interleave:
            return [(f_, len(j[1])) for fs in zip(*out) for f_, j in zip(fs, jobs)]
        return [(f_, len(j[1])) for fs, j in zip(out, jobs) for f_ in fs]

    def inv(t, R=None, W=None):
        R = R or OPT['R']
        W = W or OPT['W']
        nr = B // R
        for m in (2 * t, 2 * t + 1):
            ys = jnp.concatenate([jnp.concatenate([qs.pop(('y', m, c * nr + r)) for c in range(D // W)], axis=1)
                                  for r in range(nr)], axis=0)
            y_v[m * B:(m + 1) * B, :] = _dot(g_ref[...], pltpu.bitcast(ys, BF16))

    plan = _plan()

    def both(ws, ss, nm=[0]):
        def f_():
            nm[0] += 1
            with _scope("bar%d" % nm[0]):
                wait(ws)
            start(ss)
        return f_


    if ONLY:
        st["hprev"] = yss[0][z0]
        for tt in range(min(ONLY, 7)):
            for ph in 'AHB':
                for m, _ in plan[tt, ph]:
                    started.add(m)
    with _scope("pro_a"):
      if ONLY:
        both(inc[0][0:2], inc[2][0:3])()
        both([inc[0][3]] + small[5:], [inc[2][3], wc[3]])()
      else:
        st["fresh"] = (0,)
        fwd_h(0)
        fwd_h(1)
        both(inc[0][0:2], inc[2][0:3])()
        for m in (0, 1):
            for c in range(8):
                kv_q(m, c)
            fwd_x(m)
        both([inc[0][3]] + small[5:], [inc[2][3], wc[3]])()
        for f_, _ in pieces([(0, [0]), (1, [0, 1])], True, 8, 512):
            f_()
        inv(0, 8, 512)
        for n in range(2):
            a_layer(q_v[n * B:(n + 1) * B, :].astype(F32), y_v3[z0, n * B:(n + 1) * B, :], slice(n * B, (n + 1) * B), rs(2 * TM, n * B, B))

    def paced(seq, barriers, fill, tstart=0):
        T = sum(c for _, c, _ in seq)
        tend = T - ENDM
        at, saved, ev, now = {}, {}, [], 0
        def run_mxu(fn, kind):
            cur = st["clk"]
            st["clk"] = saved[kind]
            fn()
            st["clk"] = cur
        def save_clk(kind):
            saved[kind] = st["clk"]
        prev_emit = 0
        for fn, c, kind in seq:
            at[kind] = now
            if kind in barriers:
                ev.append((prev_emit + 1, barriers[kind], None))
                at['b' + kind] = prev_emit + 2
            ev.append((max(now - MARGIN, 0), P(save_clk, kind), None))
            prev_emit = now + LATE * c // 1024
            ev.append((prev_emit, P(run_mxu, fn, kind), None))
            now += c
        def spread(fns, t0, t1, dl):
            t1 = min(t1, tend - dl * TICK)
            fns = [f_ if isinstance(f_, tuple) else (f_, 1) for f_ in fns]
            tot = sum(w for _, w in fns)
            acc = 0
            for fn, w in fns:
                ev.append((t0 + (t1 - t0) * acc / tot, fn, dl))
                acc += w
        def stages(fn, cx, stgs, ng, t0, t1):
            t1 = t1 - (len(stgs) + 1) * SG
            for j, stg in enumerate(stgs):
                last = stg == (2 if fn is nrm_q else 4)
                off = j * SG + (SG if last else 0)
                spread([P(fn, cx, g, stg) for g in range(ng // 2 if last else ng)], t0 + off, t1 + off, LND)
        fill(at, tend, spread, stages)
        ev.sort(key=lambda e: e[0])
        ties, n = {}, 0
        for k in range(int(T / TICK) + 2):
            while n < len(ev) and ev[n][0] < (k + 1) * TICK:
                r = ev[n][1]()
                if ev[n][2] is not None:
                    ties.setdefault(k + ev[n][2], []).extend(r)
                n += 1
            c = st["clk"]
            tl = ties.pop(k + 1, None)
            if tl:
                while len(tl) > 1:
                    tl = [tl[j] | tl[j + 1] if j + 1 < len(tl) else tl[j] for j in range(0, len(tl), 2)]
                c = c | (tl[0] & zm)
            st["clk"] = pltpu.roll(c, 1, axis=1) if tstart <= (k + 1) * TICK <= tend else c
        assert n == len(ev) and not any(ties.values())

    extra = iter(range(NC))

    def norm0():
        z2a_v[HS[0], :] = _ln2(zt_v[z0]).astype(BF16)

    def region(t, order, barriers):
        conv = t + 1 < NT
        st["fresh"] = (t + 1,)
        hs = HS[t % 2] if t else HS[2]
        seq = []
        for kind in order.split():
            n = int(kind[1:] or 0)
            if kind[0] == 'h':
                seq.append((P(fwd_h, 2 * t + 2 + n), 512, kind))
            elif kind[0] == 'x':
                seq.append((P(fwd_x, 2 * t + 2 + n), 512, kind))
            elif kind[0] == 'i':
                seq.append((P(inv, t + 1), 1024, kind))
            elif kind[0] == 'e':
                seq.append((P(z1_step, HS[2], HS[0], False, next(extra)), 1024, kind))
            elif kind[0] == 'a':
                seq.append((lambda: a_layer(q_v[HS[1], :].astype(F32), y_v3[z0, HS[1], :], HS[1], HS[1]), 0, kind))
            elif kind[0] == 'n':
                seq.append((norm0, 0, kind))
            elif kind[0] == 'w':
                seq.append((lambda: None, n, kind))
            else:
                seq.append((P(z2_step, hs, HS[0], n) if n < NC else
                            P(z1_step, hs, rs(t * TM, 0, TM), False, n - NC), 1024, kind))
        def fill(at, tend, spread, stages):
            if t:
                stages(nrm_q, (z2a_v, t * TM, 0), (0, 1, 2), 32, at['s6'] + 1524, tend)
            if conv:
                t0 = at.get('bh0', 0)
                mid = (t0 + at['x1'] - 800) // 2
                spread([P(kv_q, 2 * t + 2, c) for c in range(8)], t0, min(mid, at['x0'] - 800), KVD)
                spread([P(kv_q, 2 * t + 3, c) for c in range(8)], min(mid, at['x0'] - 800), at['x1'] - 800, KVD)
                b1 = (t + 1) * TM
                cx = (q_v3, b1, b1, x_v3, b1, ((t + 1) % 2) * TM)
                if t:
                    stages(a_q, cx, (0, 1), 32, at['i'] - 3000, at['i'] + 1000)
                    stages(a_q, cx, (2, 3, 4), 32, at['i'] + 1500, tend)
                spread(pieces(plan[t, 'A'], False, fr=OPT['frA']), 0, at['x1'] + 1000, HD)
                spread(pieces(plan[t, 'H'], True, interleave=True), at['x1'] + (1000 if t else OPT['h0']), at['i'] - (700 if t else OPT['h1']), HD)
                spread(pieces(plan[t, 'B'], False, fr=OPT['frB']), at['i'] + OPT['b0'], tend, HD)
        paced(seq, barriers, fill)

    for t in range(NT):
        barriers = {}
        order = ORD.get(t, ORD[2])
        if t == 0:
            both([wc[0]], [wc[4]])()
            barriers['h0'] = both(inc[1][0:3], [])
            barriers['s3'] = both([wc[1]], [])
            barriers['i'] = both([inc[1][3], wc[2]], [])
        elif t == 1:
            both(inc[2][0:3], inc[3])()
            barriers['s4'] = both([inc[2][3], wc[3]], [])
            barriers['s10'] = both([wc[4]], [])
        elif t + 1 < NT:
            wait(inc[t + 1])
            start(inc[t + 2] if t + 2 < NT else [wsp_copy(0), wout_copies[0]])
        else:
            wsp_copy(0).wait()
            start([wsp_copy(1), wout_copies[1]])
        with _scope("p1_%d" % t):
            if ONLY is None or ONLY == t:
                region(t, order, barriers)
            else:
                for b_ in barriers.values():
                    b_()
    clk_v[...] = st["clk"]
    if ONLY is not None and ONLY < 8:
        d8 = pl.ds(pl.multiple_of(z0 * 16, 16), 16)
        acc = st["hprev"][0:16, 0:128] + pltpu.bitcast(clk_v[...], F32)[0:1]
        for b_ in list(sps) + list(yss) + [x_v3, y_v3]:
            acc = acc + b_[z0, d8, pl.ds(pl.multiple_of(z0 * 128, 128), 128)]
        for b_ in (z1_v, z2a_v, h_v):
            acc = acc + b_[d8, pl.ds(pl.multiple_of(z0 * 128, 128), 128)].astype(F32)
        q_v[0:16, 0:128] = acc.astype(BF16)
        cp = pltpu.make_async_copy(q_v, out_hbm.at[0], sem_out.at[0, 0])
        cp.start()
        cp.wait()
        wait([wsp_copy(1)] + wout_copies)
        return

    def rows1(i):
        return pl.ds(pl.multiple_of(i * TM, TM), TM)

    def uslot(i):
        return pl.ds(pl.multiple_of((i % 2) * TM, TM), TM)

    clk0 = jax.lax.broadcasted_iota(I32, (8, 128), 1) & zm
    NO = D // CN

    def p2(i, _):
        wsp_copy(i + 1).wait()

        @pl.when(i + 2 < NT)
        def _():
            wsp_copy(i + 2).start()

        st["clk"] = clk0
        base = pl.multiple_of(i * TM, TM)
        r = rows1(i)
        seq = [(P(o_step, r, uslot(i), yss[0], False, c), FH, 'o%d' % c) for c in range(NO)]
        seq += [(P(g_step, rows1(i + 1), uslot(i + 1), c), S, 'g%d' % c) for c in range(NC)]
        seq += [(P(z2_step, HS[0], HS[0], c), D, 's%d' % c) for c in range(NC)]
        seq += [(P(z1_step, HS[0], r, False, c), D, 's%d' % (NC + c)) for c in range(NC)]
        def fill(at, tend, spread, stages):
            stages(a_q, (yss[0], 0, base, yss[1], 0, 0), (0, 1, 2, 3, 4), 32, at['g0'] + OPT['a0'], at['s0'] - OPT['a1'])
            stages(nrm_q, (z2b_v, base, 0), (0, 1, 2), 32, at['s7'] + 500, tend)
        paced(seq, {}, fill, FH * NO - 2 * MARGIN)
        clk_v[...] = st["clk"]
        return 0

    with _scope("p2"):
        mm2(slice(0, TM), HS[0], z2a_v, True)
        wait(wout_copies)
        jax.lax.fori_loop(0, NT - 1, p2, 0)
        hm = TM // 2
        base = (NT - 1) * TM
        st["clk"] = clk0
        seq = []
        for n in range(2):
            seq += [(P(o_step, rs(base, n * hm, hm), rs(TM, n * hm, hm), yss[2 * n], n > 0, c), FH // 2, 'o%d%d' % (n, c))
                    for c in range(NO)]
        for n in range(2):
            hs = rs(0, n * hm, hm)
            seq += [(P(z2_step, hs, hs, c), D // 2, 's%d%d' % (n, c)) for c in range(NC)]
            seq += [(P(z1_step, hs, rs(base, n * hm, hm), False, c), D // 2, 't%d%d' % (n, c)) for c in range(NC)]
        def fill(at, tend, spread, stages):
            stages(a_q, (yss[0], 0, base, yss[1], 0, 0), (0, 1, 2, 3, 4), 16, at['o10'] + 300, at['s00'] - 200)
            stages(a_q, (yss[2], 0, base + hm, yss[3], 0, hm), (0, 1, 2, 3, 4), 16, at['s00'] + 300, at['t00'] + 300)
            stages(nrm_q, (z2b_v, base, 0), (0, 1, 2), 16, at['t00'] + 400, at['s10'])
            stages(nrm_q, (z2b_v, base + hm, hm), (0, 1, 2), 16, at['t10'] + 400, tend)
        paced(seq, {}, fill, FH * NO // 2 - 2 * MARGIN)
        clk_v[...] = st["clk"]

    o_v = q_v
    def rows2(i):
        r0 = pl.multiple_of(i * (2 * TM), 2 * TM)
        return pl.ds(r0, TM), pl.ds(r0 + TM, TM)

    def out_copies(i):
        ra, rb = rows2(i)
        hd = D // 2
        return [pltpu.make_async_copy(o_v.at[ra], out_hbm.at[0, ra], sem_out.at[i, 0]),
                pltpu.make_async_copy(o_v.at[rb, 0:hd], out_hbm.at[0, rb, 0:hd], sem_out.at[i, 1]),
                pltpu.make_async_copy(o_v.at[rb, hd:D], out_hbm.at[0, rb, hd:D], sem_out.at[i, 2])]

    def p3(i, _):
        ra, rb = rows2(i)
        oc = out_copies(i)
        mm2(ra, HS[0], z2b_v, True)
        mm2(rb, HS[1], z2b_v, True)
        o_v[ra, :] = mm3(ra, HS[0]).astype(BF16)
        oc[0].start()
        for n in range(2):
            cs = slice(n * (D // 2), (n + 1) * (D // 2))
            o_v[rb, cs] = (x_v[rb, cs] + _dot(u_v[HS[1], :], wout_v[:, cs])).astype(BF16)
            oc[1 + n].start()
        return 0

    with _scope("p3"):
        jax.lax.fori_loop(0, NT // 2, p3, 0)
    with _scope("outwait"):
        for i in range(NT // 2):
            wait(out_copies(i))


@jax.jit
def pallas_interleave_layers__ssm_conv_h3__mixer_gmlp__prompt_kernel(A_q, A_k, A_v, A_shift_k, A_ssm_k, A_ssm_D, B_x, B_w_in, B_w_sp, B_b_sp, B_w_out):
    f, g = _dft_mats()
    any_ = pl.BlockSpec(memory_space=pl.ANY)
    return pl.pallas_call(
        kernel,
        out_shape=jax.ShapeDtypeStruct((1, S, D), BF16),
        in_specs=[any_] * 13,
        out_specs=any_,
        scratch_shapes=[
            pltpu.VMEM((D, F), BF16), pltpu.VMEM((S, S), BF16), pltpu.VMEM((FH, D), BF16),
            pltpu.VMEM((S, FH), F32), pltpu.VMEM((S, FH), BF16),
            pltpu.VMEM((1, S, D), F32), pltpu.VMEM((1, S, D), F32),
            pltpu.VMEM((3 * TM, D), BF16), pltpu.VMEM((1, S, D), BF16),
            pltpu.VMEM((S, 128), F32),
            pltpu.VMEM((S, 2 * D), BF16), pltpu.VMEM((D, S), BF16),
            pltpu.VMEM((1, TM, FH), F32), pltpu.VMEM((4, D), F32), pltpu.VMEM((8, 128), I32),
            pltpu.VMEM((4, D), BF16), pltpu.VMEM((D,), BF16), pltpu.VMEM((S,), BF16),
            pltpu.VMEM((2 * B, B), BF16), pltpu.VMEM((B, 2 * B), BF16), pltpu.SMEM((1,), I32),
            pltpu.SemaphoreType.DMA((NT, 4)), pltpu.SemaphoreType.DMA((7 + NT,)), pltpu.SemaphoreType.DMA((6,)),
            pltpu.SemaphoreType.DMA((NT // 2, 3)),
        ] + [pltpu.VMEM((2, B + OPT['pr'], WSP), F32)] * NT + [pltpu.VMEM((1, 2 * B, D), F32)] * NYS,
        compiler_params=pltpu.CompilerParams(vmem_limit_bytes=127 * 1024 * 1024),
    )(A_q, A_k, A_v, A_shift_k.T, A_ssm_k, A_ssm_D, B_w_in, B_w_sp, B_b_sp, B_w_out,
      jnp.asarray(f, BF16), jnp.asarray(g, BF16), jnp.asarray(np.zeros((1,), np.int32)))
```

```python
import functools
import numpy as np
import jax
import jax.numpy as jnp
import jax.experimental.pallas as pl
import jax.experimental.pallas.tpu as pltpu

S, D, F = 2048, 1024, 3584
FH = F // 2
B = 128
NB = S // B
TM = 256
NT = S // TM
EPS = 1e-5
F32, BF16, I32 = jnp.float32, jnp.bfloat16, jnp.int32
CN = 256
NC = FH // CN
OXC, OXS, OHC, OHS = 0, D + 128, 2 * (D + 128), 3 * (D + 128)
WSP = 4 * D + 3 * 128
NYS = 6
P = functools.partial
SCOPES = False
NA = {1: 5, 2: 5, 3: 7, 4: 6, 5: 4, 6: 8}
NBP = {1: 9, 2: 13, 3: 12, 4: 13, 5: 8}
PR, PW = 16, 128

ORD = {0: 's0 s1 s2 h0 h1 w600 x0 x1 s3 s4 w500 i s5 a s6 n',
       1: 's0 h0 s1 h1 s2 x0 s3 x1 s4 s5 s6 s7 i s8 e0 s9 s10 s11 e1 e2',
       2: 'e0 s0 h0 s1 h1 s2 x0 s3 x1 s4 s5 s6 s7 i s8 s9 s10 s11 s12 s13',
       4: 'e0 s0 h0 s1 h1 s2 x0 s3 x1 s4 s5 s6 s7 i s8 e1 s9 s10 s11 s12 s13',
       7: 's0 s1 s2 s3 s4 s5 s6 s7 s8 s9 s10 s11 s12 s13'}

TICK, MARGIN, LATE, ENDM = 112, 300, 700, 400
SG, LND, KVD, HD = 330, 3, 3, 2


def _dft_mats():
    ks = np.concatenate([np.arange(0, B, 2), np.arange(1, B, 2)])
    th = np.pi * (2 * ks + 1) / (2 * B)
    n = np.arange(B)
    ang = th[:, None] * n[None, :]
    f = np.concatenate([np.cos(ang), np.sin(ang)], axis=0)
    g = np.empty((B, 2 * B))
    g[:, 0::2] = np.cos(ang).T / B
    g[:, 1::2] = np.sin(ang).T / B
    return f.astype(np.float32), g.astype(np.float32)


def _plan():
    done = {(0, 0), (1, 0), (1, 1)}
    plan = {}
    def take(key, pairs):
        jobs = {}
        for m, i in pairs:
            done.add((m, i))
            jobs.setdefault(m, []).append(i)
        plan[key] = sorted(jobs.items())
    pend = []
    for t in range(NT - 1):
        take((t, 'A'), pend)
        take((t, 'H'), [(m, i) for m in (2 * t + 2, 2 * t + 3) for i in range(m + 1) if (m, i) not in done])
        a = 2 * t + 3
        cand = [(m, i) for m in range(2 * t + 4, min(2 * t + 4 + NYS, NB)) for i in range(m + 1)
                if i <= a and m - i <= a and (m, i) not in done]
        nb, na = NBP.get(t, 0), NA.get(t + 1, 0)
        take((t, 'B'), cand[:nb])
        pend = cand[nb:nb + na]
        for c in pend:
            done.add(c)
    assert len(done) == NB * (NB + 1) // 2
    return plan


def _ln(x):
    m = jnp.mean(x, axis=-1, keepdims=True)
    xc = x - m
    v = jnp.mean(xc * xc, axis=-1, keepdims=True)
    return xc * jax.lax.rsqrt(v + EPS)


def _ln2(x):
    m = jnp.mean(x, axis=-1, keepdims=True)
    xc = x - m
    v = jnp.mean(xc * xc, axis=-1, keepdims=True)
    return xc * (0.5 * jax.lax.rsqrt(v + 4 * EPS))


def _gelu(x):
    c = np.float32(np.sqrt(2.0 / np.pi))
    inner = x * (c + (c * np.float32(0.044715)) * (x * x))
    return x + x * jnp.tanh(inner)


def _dot(a, b):
    return jnp.dot(a, b, preferred_element_type=F32)


class _NoScope:
    def __enter__(self): return self
    def __exit__(self, *a): return False


def _scope(name):
    return jax.named_scope(name) if SCOPES else _NoScope()


def kernel(q_hbm, k_hbm, v_hbm, shk_hbm, sk_hbm, sd_hbm, win_hbm, wsp_hbm, bsp_hbm, wout_hbm,
           f_hbm, g_hbm, zs_hbm, out_hbm,
           win_v, wsp_v, wout_v, z1_v, z2a_v, x_v3, y_v3, h_v, q_v3, bb_v,
           kv_v, sk_v, zt_v, shk_v, clk_v, shk_ref, sd_ref, bsp_ref, f_ref, g_ref, zs_ref,
           sem_in, sem_w, sem_s, sem_out, *bufs):
    sps, yss = bufs[:NT], bufs[NT:]
    x_v, y_v, q_v = x_v3.at[0], y_v3.at[0], q_v3.at[0]
    k_v = kv_v.at[:, 0:D]
    v_v = kv_v.at[:, D:2 * D]
    z2b_v = kv_v.at[:, 0:FH]
    u_v = sk_v.at[0:2 * TM, 0:FH]
    HS = [slice(n * TM, (n + 1) * TM) for n in range(4)]

    bi = lambda x: pltpu.bitcast(x, I32)
    hi = lambda w: pltpu.bitcast(w & np.int32(-65536), F32)
    lo = lambda w: pltpu.bitcast(w << 16, F32)
    pk = lambda a, b: bi(pltpu.pack_elementwise([a, b], packed_dtype=BF16))
    bc = lambda m: jnp.broadcast_to(m, (m.shape[0], 128))
    wide = lambda m, n: jnp.concatenate([m] * n, axis=1)
    rows8 = lambda x: [x[r:r + 8, c:c + 128] for r in range(0, x.shape[0], 8) for c in range(0, x.shape[1], 128)]
    half = lambda sl: slice(sl.start // 2, sl.stop // 2)
    cols = lambda x: [x[:, c:c + 128] for c in range(0, x.shape[1], 128)]

    WG = ((FH, FH + 3 * CN), (FH + 3 * CN, FH + 5 * CN), (FH + 5 * CN, F), (0, 5 * CN), (5 * CN, FH))
    wc = [pltpu.make_async_copy(win_hbm.at[:, a:b], win_v.at[:, a:b], sem_w.at[n]) for n, (a, b) in enumerate(WG)]
    def wsp_copy(n):
        r = pl.ds(pl.multiple_of(n * TM, TM), TM)
        return pltpu.make_async_copy(wsp_hbm.at[r], wsp_v.at[r], sem_w.at[7 + n])
    wout_copies = [pltpu.make_async_copy(wout_hbm.at[n * (FH // 2):(n + 1) * (FH // 2)],
                                         wout_v.at[n * (FH // 2):(n + 1) * (FH // 2)], sem_w.at[5 + n]) for n in range(2)]
    small = [pltpu.make_async_copy(a, b, sem_s.at[n]) for n, (a, b) in enumerate(
        [(zs_hbm, zs_ref), (f_hbm, f_ref), (shk_hbm, shk_ref), (sd_hbm, sd_ref), (bsp_hbm, bsp_ref), (g_hbm, g_ref)])]

    def tile_copies(t):
        r = pl.ds(t * TM, TM)
        return [pltpu.make_async_copy(k_hbm.at[0, r], k_v.at[r], sem_in.at[t, 0]),
                pltpu.make_async_copy(v_hbm.at[0, r], v_v.at[r], sem_in.at[t, 1]),
                pltpu.make_async_copy(sk_hbm.at[:, r], sk_v.at[:, r], sem_in.at[t, 2]),
                pltpu.make_async_copy(q_hbm.at[0, r], q_v.at[r], sem_in.at[t, 3])]
    inc = [tile_copies(t) for t in range(NT)]

    def start(cs):
        for c in cs:
            c.start()

    def wait(cs):
        for c in cs:
            c.wait()

    def a_layer(x, y, rows, hs):
        x1 = x + _ln(x) * y
        x_v[rows, :] = x1
        h_v[half(hs), :] = bi(_ln(x1).astype(BF16))

    def mm2(rows, hs, z2_src, act=False):
        bb = wide(bb_v[rows, :], CN // 128)
        for c in range(NC):
            cs = slice(c * CN, (c + 1) * CN)
            g = _dot(wsp_v[rows, :], pltpu.bitcast(z2_src[:, cs], BF16)) + bb
            z1 = z1_v[rows, cs]
            u_v[hs, cs] = ((_gelu(z1) if act else z1) * g).astype(BF16)

    def mm3(rows, hs):
        return x_v[rows, :] + _dot(u_v[hs, :], wout_v[...])

    with _scope("pro_init"):
        first = small[0:5] + inc[0][2:3]
        start(first)
        for sm, grp in zip(first, (inc[0][0:2] + small[5:], [inc[0][3], wc[0]], inc[1][0:3], [wc[1]], [inc[1][3]],
                                   [wc[2]])):
            sm.wait()
            start(grp)
    z0 = zs_ref[0]
    dz = [z0 * k for k in range(4)]
    zm = jnp.full((8, 128), z0, I32)
    with _scope("pro_bb"):
        shk_v[...] = shk_ref[...].astype(F32)
        bb_v[...] = jnp.transpose(jnp.broadcast_to(0.5 * bsp_ref[...].astype(F32).reshape(1, S), (128, S)))

    st = {"hprev": None, "clk": jax.lax.broadcasted_iota(I32, (8, 128), 1) & zm}
    qs = {}
    started = set()

    def lnk(h):
        h00 = pltpu.bitcast(bi(h[0:16, 0:128]) | st["clk"], BF16)
        return jnp.concatenate([jnp.concatenate([h00, h[0:16, 128:]], axis=1), h[16:]], axis=0)

    def lhs(hs):
        w = h_v[half(hs), :]
        w0 = jnp.concatenate([w[0:8, 0:128] | st["clk"], w[0:8, 128:]], axis=1)
        return pltpu.bitcast(jnp.concatenate([w0, w[8:]], axis=0), BF16)

    def rs(base, off, n):
        if isinstance(base, int):
            return slice(base + off, base + off + n)
        return pl.ds(pl.multiple_of(base + off, n), n)

    def z2_step(hs, zr, c):
        zt_v[0, zr, c * CN:(c + 1) * CN] = _gelu(_dot(lhs(hs), win_v[:, FH + c * CN:FH + (c + 1) * CN]))

    def z1_step(hs, rows, act, c):
        z = _dot(lhs(hs), win_v[:, c * CN:(c + 1) * CN])
        z1_v[rows, c * CN:(c + 1) * CN] = _gelu(z) if act else z

    def g_step(rows, us, c):
        cs = slice(c * CN, (c + 1) * CN)
        g = _dot(lnk(wsp_v[rows, :]), pltpu.bitcast(z2a_v[:, cs], BF16)) + wide(bb_v[rows, :], CN // 128)
        u_v[us, cs] = (_gelu(z1_v[rows, cs]) * g).astype(BF16)

    def o_step(rows, us, xt, link, c):
        cs = slice(c * CN, (c + 1) * CN)
        u = u_v[us, :]
        xt[0, 0:u.shape[0], cs] = x_v[rows, cs] + _dot(lnk(u) if link else u, wout_v[:, cs])

    def ssum(xs):
        s_ = xs[0]
        for v in xs[1:]:
            s_ = s_ + v
        return jnp.sum(s_, axis=-1, keepdims=True) * (1.0 / (128 * len(xs)))

    def st_mean(key, x):
        m = qs[key] = bc(ssum(cols(x)))
        return [bi(m)]

    def st_rstd(key, mkey, x, half=False):
        m = qs[mkey]
        xc = [v - m for v in cols(x)]
        r = jax.lax.rsqrt(ssum([v * v for v in xc]) + (4 * EPS if half else EPS))
        r = qs[key] = bc(0.5 * r if half else r)
        return [bi(r)]

    def st_out(dst, r0, gp, ld, w, mkey, rkey):
        g, p = gp // 2, gp % 2
        cs = slice(p * w // 2, (p + 1) * w // 2)
        x = ld(g, cs)
        n = x.shape[1] // 128
        m = jnp.concatenate([pltpu.bitcast(bi(qs[mkey, 2 * g + j]) | st["clk"], F32) for j in range(2)], axis=0)
        r = jnp.concatenate([qs[rkey, 2 * g + j] for j in range(2)], axis=0)
        o = ((x - wide(m, n)) * wide(r, n)).astype(BF16)
        if dst is h_v or dst is z2a_v:
            dst[half(rs(r0, 16 * g, 16)), cs] = bi(o)
        else:
            dst[rs(r0, 16 * g, 16), cs] = o
        return []

    def nrm_q(cx, g, stage):
        dst, base, z0r = cx
        if stage == 0:
            return st_mean(('nm', g), zt_v[dz[1], rs(z0r, 8 * g, 8), :])
        if stage == 1:
            return st_rstd(('nr', g), ('nm', g), zt_v[dz[2], rs(z0r, 8 * g, 8), :], True)
        return st_out(dst, base, g, lambda g, cs: zt_v[dz[3], rs(z0r, 16 * g, 16), cs], FH, 'nm', 'nr')

    def a_q(cx, g, stage):
        src, s0, base, xs, x0, h0 = cx
        r = rs(base, 8 * g, 8)
        if stage <= 2:
            x = src[dz[stage + 1], rs(s0, 8 * g, 8), :].astype(F32)
        if stage == 0:
            return st_mean(('am', g), x)
        if stage == 1:
            return st_rstd(('ar', g), ('am', g), x)
        if stage == 2:
            x1 = x + ((x - wide(qs['am', g], 8)) * wide(qs['ar', g], 8)) * y_v3[dz[1], r, :]
            x_v[r, :] = x1
            if xs is not x_v3:
                xs[0, rs(x0, 8 * g, 8), :] = x1
            return st_mean(('am', g), x1)
        if stage == 3:
            return st_rstd(('ar', g), ('am', g), xs[0, rs(x0, 8 * g, 8), :])
        return st_out(h_v, h0, g, lambda g, cs: xs[0, rs(x0, 16 * g, 16), cs], D, 'am', 'ar')

    def kv_q(m, c):
        cs = slice(c * 128, (c + 1) * 128)
        if m == 0:
            kw = jnp.concatenate([jnp.zeros((8, 128), I32), bi(k_v[0:B, cs])], axis=0)
        else:
            kw = bi(k_v[m * B - 16:(m + 1) * B, cs])
        k0 = kw[8:]
        k1 = pltpu.roll(kw, 1, axis=0)[8:]
        k2 = pltpu.roll(kw, 2, axis=0)[8:]
        w = [jnp.broadcast_to(shk_v[j:j + 1, cs], (8, 128)) for j in range(4)]
        vw = bi(v_v[m * B:(m + 1) * B, cs])
        out = []
        for n in range(8):
            r = slice(8 * n, 8 * n + 8)
            e0, o0, e1, o1, o2 = lo(k0[r]), hi(k0[r]), lo(k1[r]), hi(k1[r]), hi(k2[r])
            w0 = w[0] if (not out or m < 2) else pltpu.bitcast(bi(w[0]) | (out[-1] & zm), F32)
            se = ((e0 * w0 + o1 * w[1]) + e1 * w[2]) + o2 * w[3]
            so = ((o0 * w0 + e0 * w[1]) + o1 * w[2]) + e1 * w[3]
            out.append(pk(se * lo(vw[r]), so * hi(vw[r])))
        qs['kv', m, c] = jnp.concatenate(out, axis=0)
        return [out[-1]]

    def fwd_x(m):
        kvb = pltpu.bitcast(jnp.concatenate([qs.pop(('kv', m, c)) for c in range(8)], axis=1), BF16)
        xf = _dot(f_ref[...], kvb)
        sps[m // 2][m % 2, 0:B, OXC:OXC + D] = xf[0:B]
        sps[m // 2][m % 2, 0:B, OXS:OXS + D] = xf[B:2 * B]
        if m % 2:
            sps[m // 2][z0, 0:8, D:D + 128] = jnp.zeros((8, 128), F32)

    def fwd_h(m):
        hraw = jax.lax.dot_general(f_ref[...], sk_v[:, m * B:(m + 1) * B], (((1,), (1,)), ((), ())),
                                   preferred_element_type=F32)
        hprev = st["hprev"]
        hb = B // 2
        sp = sps[m // 2]
        if hprev is None:
            hraw = jnp.concatenate([hraw[0:B] + sd_ref[...].astype(F32).reshape(1, D), hraw[B:2 * B]], axis=0)
            sp[m % 2, 0:B, OHC:OHC + D] = hraw[0:B]
            sp[m % 2, 0:B, OHS:OHS + D] = hraw[B:2 * B]
        else:
            sp[m % 2, 0:hb, OHC:OHC + D] = hraw[0:hb] + hprev[B:B + hb]
            sp[m % 2, hb:B, OHC:OHC + D] = hraw[hb:B] - hprev[B + hb:2 * B]
            sp[m % 2, 0:hb, OHS:OHS + D] = hraw[B:B + hb] - hprev[0:hb]
            sp[m % 2, hb:B, OHS:OHS + D] = hraw[B + hb:2 * B] + hprev[hb:B]
        st["hprev"] = hraw

    def piece(m, iis, acc, final, R, W, p):
        nr = B // R
        r0 = (p % nr) * R
        c0 = (p // nr) * W
        ys = yss[m % NYS]
        yr = yi = None
        if acc:
            yr = ys[0, r0:r0 + R, c0:c0 + W]
            yi = ys[0, B + r0:B + r0 + R, c0:c0 + W]
        def ld(b, off):
            return sps[b // 2][b % 2, r0:r0 + R, off + c0:off + c0 + W]
        for i in iis:
            xr, xi, hr, hi_ = ld(i, OXC), ld(i, OXS), ld(m - i, OHC), ld(m - i, OHS)
            yr = (xr * hr if yr is None else yr + xr * hr) - xi * hi_
            yi = (xr * hi_ if yi is None else yi + xr * hi_) + xi * hr
        if final:
            r_ = qs['y', m, p] = pk(yr, yi)
            return rows8(r_)
        ys[0, r0:r0 + R, c0:c0 + W] = yr
        ys[0, B + r0:B + r0 + R, c0:c0 + W] = yi
        return rows8(bi(yr) | bi(yi))

    def pieces(jobs, final, R=PR, W=PW, interleave=False):
        out = []
        for m, iis in jobs:
            out.append([P(piece, m, iis, m in started, final, R, W, p) for p in range((B // R) * (D // W))])
            started.add(m)
        if interleave:
            return [(f_, len(j[1])) for fs in zip(*out) for f_, j in zip(fs, jobs)]
        return [(f_, len(j[1])) for fs, j in zip(out, jobs) for f_ in fs]

    def inv(t, R=PR, W=PW):
        nr = B // R
        for m in (2 * t, 2 * t + 1):
            ys = jnp.concatenate([jnp.concatenate([qs.pop(('y', m, c * nr + r)) for c in range(D // W)], axis=1)
                                  for r in range(nr)], axis=0)
            y_v[m * B:(m + 1) * B, :] = _dot(g_ref[...], pltpu.bitcast(ys, BF16))

    plan = _plan()

    def both(ws, ss, nm=[0]):
        def f_():
            nm[0] += 1
            with _scope("bar%d" % nm[0]):
                wait(ws)
            start(ss)
        return f_


    with _scope("pro_a"):
        fwd_h(0)
        fwd_h(1)
        both(inc[0][0:2], inc[2])()
        for m in (0, 1):
            for c in range(8):
                kv_q(m, c)
            fwd_x(m)
        both([inc[0][3]] + small[5:], [wc[3]])()
        for f_, _ in pieces([(0, [0]), (1, [0, 1])], True, 8, 512):
            f_()
        inv(0, 8, 512)
        for n in range(2):
            a_layer(q_v[n * B:(n + 1) * B, :].astype(F32), y_v3[z0, n * B:(n + 1) * B, :], slice(n * B, (n + 1) * B), rs(2 * TM, n * B, B))

    def paced(seq, barriers, fill, tstart=0):
        T = sum(c for _, c, _ in seq)
        tend = T - ENDM
        at, saved, ev, now = {}, {}, [], 0
        def run_mxu(fn, kind):
            cur = st["clk"]
            st["clk"] = saved[kind]
            fn()
            st["clk"] = cur
        def save_clk(kind):
            saved[kind] = st["clk"]
        prev_emit = 0
        for fn, c, kind in seq:
            at[kind] = now
            if kind in barriers:
                ev.append((prev_emit + 1, barriers[kind], None))
                at['b' + kind] = prev_emit + 2
            ev.append((max(now - MARGIN, 0), P(save_clk, kind), None))
            prev_emit = now + LATE * c // 1024
            ev.append((prev_emit, P(run_mxu, fn, kind), None))
            now += c
        def spread(fns, t0, t1, dl):
            t1 = min(t1, tend - dl * TICK)
            fns = [f_ if isinstance(f_, tuple) else (f_, 1) for f_ in fns]
            tot = sum(w for _, w in fns)
            acc = 0
            for fn, w in fns:
                ev.append((t0 + (t1 - t0) * acc / tot, fn, dl))
                acc += w
        def stages(fn, cx, stgs, ng, t0, t1):
            t1 = t1 - (len(stgs) + 1) * SG
            for j, stg in enumerate(stgs):
                last = stg == (2 if fn is nrm_q else 4)
                off = j * SG + (SG if last else 0)
                spread([P(fn, cx, g, stg) for g in range(ng)], t0 + off, t1 + off, LND)
        fill(at, tend, spread, stages)
        ev.sort(key=lambda e: e[0])
        ties, n = {}, 0
        for k in range(int(T / TICK) + 2):
            while n < len(ev) and ev[n][0] < (k + 1) * TICK:
                r = ev[n][1]()
                if ev[n][2] is not None:
                    ties.setdefault(k + ev[n][2], []).extend(r)
                n += 1
            c = st["clk"]
            tl = ties.pop(k + 1, None)
            if tl:
                while len(tl) > 1:
                    tl = [tl[j] | tl[j + 1] if j + 1 < len(tl) else tl[j] for j in range(0, len(tl), 2)]
                c = c | (tl[0] & zm)
            st["clk"] = pltpu.roll(c, 1, axis=1) if tstart <= (k + 1) * TICK <= tend else c
        assert n == len(ev) and not any(ties.values())

    extra = iter([(0, c) for c in range(NC)] + [(1, NC - 2), (1, NC - 1)])

    def norm0():
        z2a_v[half(HS[0]), :] = bi(_ln2(zt_v[z0]).astype(BF16))

    def region(t, order, barriers):
        conv = t + 1 < NT
        hs = HS[t % 2] if t > 1 else HS[2 + t]
        seq = []
        for kind in order.split():
            n = int(kind[1:] or 0)
            if kind[0] == 'h':
                seq.append((P(fwd_h, 2 * t + 2 + n), 512, kind))
            elif kind[0] == 'x':
                seq.append((P(fwd_x, 2 * t + 2 + n), 512, kind))
            elif kind[0] == 'i':
                seq.append((P(inv, t + 1), 1024, kind))
            elif kind[0] == 'e':
                te, c = next(extra)
                seq.append((P(z1_step, HS[2 + te], HS[te], False, c), 1024, kind))
            elif kind[0] == 'a':
                seq.append((lambda: a_layer(q_v[HS[1], :].astype(F32), y_v3[z0, HS[1], :], HS[1], HS[3]), 0, kind))
            elif kind[0] == 'n':
                seq.append((norm0, 0, kind))
            elif kind[0] == 'w':
                seq.append((lambda: None, n, kind))
            else:
                seq.append((P(z2_step, hs, HS[0], n) if n < NC else
                            P(z1_step, hs, rs(t * TM, 0, TM), False, n - NC), 1024, kind))
        def fill(at, tend, spread, stages):
            if t:
                stages(nrm_q, (z2a_v, t * TM, 0), (0, 1, 2), 32, at['s6'] + 1524, tend)
            if conv:
                t0 = at.get('bh0', 0)
                mid = (t0 + at['x1'] - 800) // 2
                spread([P(kv_q, 2 * t + 2, c) for c in range(8)], t0, min(mid, at['x0'] - 800), KVD)
                spread([P(kv_q, 2 * t + 3, c) for c in range(8)], min(mid, at['x0'] - 800), at['x1'] - 800, KVD)
                b1 = (t + 1) * TM
                cx = (q_v3, b1, b1, x_v3, b1, ((t + 1) % 2) * TM)
                if t:
                    stages(a_q, cx, (0, 1), 32, at['i'] - 3000, at['i'] + 1000)
                    stages(a_q, cx, (2, 3, 4), 32, at['i'] + 1500, tend)
                spread(pieces(plan[t, 'A'], False), 0, at['x1'] + 1000, HD)
                spread(pieces(plan[t, 'H'], True, interleave=True), at['x1'] + (1000 if t else 520), at['i'] - (700 if t else 300), HD)
                spread(pieces(plan[t, 'B'], False), at['i'] - 700, tend, HD)
        paced(seq, barriers, fill)

    for t in range(NT):
        barriers = {}
        order = ORD.get(t, ORD[2])
        if t == 0:
            both([wc[0]], [wc[4]])()
            barriers['h0'] = both(inc[1][0:3], [])
            barriers['x1'] = both([wc[1]], [])
            barriers['i'] = both([inc[1][3], wc[2]], [])
        elif t == 1:
            both(inc[2], inc[3])()
            barriers['x1'] = both([wc[3]], [])
        elif t + 1 < NT:
            wait(inc[t + 1] + ([wc[4]] if t == 2 else []) + ([wsp_copy(0)] if t == NT - 2 else []))
            start(inc[t + 2] + ([wsp_copy(0)] if t == NT - 3 else []) if t + 2 < NT else [wsp_copy(1)] + wout_copies)
        with _scope("p1_%d" % t):
            region(t, order, barriers)
    clk_v[...] = st["clk"]

    def rows1(i):
        return pl.ds(pl.multiple_of(i * TM, TM), TM)

    clk0 = jax.lax.broadcasted_iota(I32, (8, 128), 1) & zm
    NO = D // CN

    def p2(i, _):
        wsp_copy(i + 1).wait()

        @pl.when(i + 2 < NT)
        def _():
            wsp_copy(i + 2).start()

        st["clk"] = clk0
        base = pl.multiple_of(i * TM, TM)
        r = rows1(i)
        seq = [(P(o_step, r, HS[0], yss[0], False, c), FH, 'o%d' % c) for c in range(NO)]
        seq += [(P(g_step, rows1(i + 1), HS[0], c), S, 'g%d' % c) for c in range(NC)]
        seq += [(P(z2_step, HS[0], HS[0], c), D, 's%d' % c) for c in range(NC)]
        seq += [(P(z1_step, HS[0], r, False, c), D, 's%d' % (NC + c)) for c in range(NC)]
        def fill(at, tend, spread, stages):
            stages(a_q, (yss[0], 0, base, yss[1], 0, 0), (0, 1, 2, 3, 4), 32, at['g0'] + 1000, at['s0'] - 1500)
            stages(nrm_q, (z2b_v, base, 0), (0, 1, 2), 32, at['s7'] + 500, tend)
        paced(seq, {}, fill, FH * NO - 2 * MARGIN)
        clk_v[...] = st["clk"]
        return 0

    with _scope("p2"):
        mm2(slice(0, TM), HS[0], z2a_v, True)
        wait(wout_copies)
        with _scope("p2loop"):
            jax.lax.fori_loop(0, NT - 1, p2, 0)
        hm = TM // 2
        base = (NT - 1) * TM
        st["clk"] = clk0
        seq = []
        for n in range(2):
            seq += [(P(o_step, rs(base, n * hm, hm), rs(0, n * hm, hm), yss[2 * n], n > 0, c), FH // 2, 'o%d%d' % (n, c))
                    for c in range(NO)]
        for n in range(2):
            hs = rs(0, n * hm, hm)
            seq += [(P(z2_step, hs, hs, c), D // 2, 's%d%d' % (n, c)) for c in range(NC)]
            seq += [(P(z1_step, hs, rs(base, n * hm, hm), False, c), D // 2, 't%d%d' % (n, c)) for c in range(NC)]
        def fill(at, tend, spread, stages):
            stages(a_q, (yss[0], 0, base, yss[1], 0, 0), (0, 1, 2, 3, 4), 16, at['o10'] + 300, at['s00'] - 200)
            stages(a_q, (yss[2], 0, base + hm, yss[3], 0, hm), (0, 1, 2, 3, 4), 16, at['s00'] + 300, at['t00'] + 300)
            stages(nrm_q, (z2b_v, base, 0), (0, 1, 2), 16, at['t00'] + 400, at['s10'])
            stages(nrm_q, (z2b_v, base + hm, hm), (0, 1, 2), 16, at['t10'] + 400, tend)
        paced(seq, {}, fill, FH * NO // 2 - 2 * MARGIN)
        clk_v[...] = st["clk"]

    o_v = q_v
    def rows2(i):
        r0 = pl.multiple_of(i * (2 * TM), 2 * TM)
        return pl.ds(r0, TM), pl.ds(r0 + TM, TM)

    def out_copies(i):
        ra, rb = rows2(i)
        hd = D // 2
        return [pltpu.make_async_copy(o_v.at[ra], out_hbm.at[0, ra], sem_out.at[i, 0]),
                pltpu.make_async_copy(o_v.at[rb, 0:hd], out_hbm.at[0, rb, 0:hd], sem_out.at[i, 1]),
                pltpu.make_async_copy(o_v.at[rb, hd:D], out_hbm.at[0, rb, hd:D], sem_out.at[i, 2])]

    def p3(i, _):
        ra, rb = rows2(i)
        oc = out_copies(i)
        mm2(ra, HS[0], z2b_v, True)
        mm2(rb, HS[1], z2b_v, True)
        o_v[ra, :] = mm3(ra, HS[0]).astype(BF16)
        oc[0].start()
        for n in range(2):
            cs = slice(n * (D // 2), (n + 1) * (D // 2))
            o_v[rb, cs] = (x_v[rb, cs] + _dot(u_v[HS[1], :], wout_v[:, cs])).astype(BF16)
            oc[1 + n].start()
        return 0

    with _scope("p3"):
        jax.lax.fori_loop(0, NT // 2, p3, 0)
    with _scope("outwait"):
        for i in range(NT // 2):
            wait(out_copies(i))


@jax.jit
def pallas_interleave_layers__ssm_conv_h3__mixer_gmlp__prompt_kernel(A_q, A_k, A_v, A_shift_k, A_ssm_k, A_ssm_D, B_x, B_w_in, B_w_sp, B_b_sp, B_w_out):
    f, g = _dft_mats()
    any_ = pl.BlockSpec(memory_space=pl.ANY)
    return pl.pallas_call(
        kernel,
        out_shape=jax.ShapeDtypeStruct((1, S, D), BF16),
        in_specs=[any_] * 13,
        out_specs=any_,
        scratch_shapes=[
            pltpu.VMEM((D, F), BF16), pltpu.VMEM((S, S), BF16), pltpu.VMEM((FH, D), BF16),
            pltpu.VMEM((S, FH), F32), pltpu.VMEM((S // 2, FH), I32),
            pltpu.VMEM((1, S, D), F32), pltpu.VMEM((1, S, D), F32),
            pltpu.VMEM((2 * TM, D), I32), pltpu.VMEM((1, S, D), BF16),
            pltpu.VMEM((S, 128), F32),
            pltpu.VMEM((S, 2 * D), BF16), pltpu.VMEM((D, S), BF16),
            pltpu.VMEM((1, TM, FH), F32), pltpu.VMEM((4, D), F32), pltpu.VMEM((8, 128), I32),
            pltpu.VMEM((4, D), BF16), pltpu.VMEM((D,), BF16), pltpu.VMEM((S,), BF16),
            pltpu.VMEM((2 * B, B), BF16), pltpu.VMEM((B, 2 * B), BF16), pltpu.SMEM((1,), I32),
            pltpu.SemaphoreType.DMA((NT, 4)), pltpu.SemaphoreType.DMA((7 + NT,)), pltpu.SemaphoreType.DMA((6,)),
            pltpu.SemaphoreType.DMA((NT // 2, 3)),
        ] + [pltpu.VMEM((2, B, WSP), F32)] * NT + [pltpu.VMEM((1, 2 * B, D), F32)] * NYS,
        compiler_params=pltpu.CompilerParams(vmem_limit_bytes=127 * 1024 * 1024),
    )(A_q, A_k, A_v, A_shift_k.T, A_ssm_k, A_ssm_D, B_w_in, B_w_sp, B_b_sp, B_w_out,
      jnp.asarray(f, BF16), jnp.asarray(g, BF16), jnp.asarray(np.zeros((1,), np.int32)))
```

```python
import functools
import numpy as np
import jax
import jax.numpy as jnp
import jax.experimental.pallas as pl
import jax.experimental.pallas.tpu as pltpu

S, D, F = 2048, 1024, 3584
FH = F // 2
B = 128
NB = S // B
TM = 256
NT = S // TM
EPS = 1e-5
F32, BF16, I32 = jnp.float32, jnp.bfloat16, jnp.int32
CN = 256
NC = FH // CN
OXC, OXS, OHC, OHS = 0, D + 128, 2 * (D + 128), 3 * (D + 128)
WSP = 4 * D + 3 * 128
NYS = 6
P = functools.partial
SCOPES = False
NA = {1: 5, 2: 5, 3: 7, 4: 6, 5: 4, 6: 8}
NBP = {1: 9, 2: 13, 3: 12, 4: 13, 5: 8}
PR, PW = 16, 128

ORD = {0: 'h0 h1 w600 x0 x1 s0 s1 w500 i s2 a s3 s4 s5 s6 n',
       1: 's0 h0 s1 h1 s2 x0 s3 x1 s4 s5 s6 s7 i s8 e0 s9 s10 s11 e1 e2',
       2: 'e0 s0 h0 s1 h1 s2 x0 s3 x1 s4 s5 s6 s7 i s8 s9 s10 s11 s12 s13',
       4: 'e0 s0 h0 s1 h1 s2 x0 s3 x1 s4 s5 s6 s7 i s8 e1 s9 s10 s11 s12 s13',
       7: 's0 s1 s2 s3 s4 s5 s6 s7 s8 s9 s10 s11 s12 s13'}

TICK, MARGIN, LATE, ENDM = 112, 300, 700, 400
SG, LND, KVD, HD = 330, 3, 3, 2


def _dft_mats():
    ks = np.concatenate([np.arange(0, B, 2), np.arange(1, B, 2)])
    th = np.pi * (2 * ks + 1) / (2 * B)
    n = np.arange(B)
    ang = th[:, None] * n[None, :]
    f = np.concatenate([np.cos(ang), np.sin(ang)], axis=0)
    g = np.empty((B, 2 * B))
    g[:, 0::2] = np.cos(ang).T / B
    g[:, 1::2] = np.sin(ang).T / B
    return f.astype(np.float32), g.astype(np.float32)


def _plan():
    done = {(0, 0), (1, 0), (1, 1)}
    plan = {}
    def take(key, pairs):
        jobs = {}
        for m, i in pairs:
            done.add((m, i))
            jobs.setdefault(m, []).append(i)
        plan[key] = sorted(jobs.items())
    pend = []
    for t in range(NT - 1):
        take((t, 'A'), pend)
        take((t, 'H'), [(m, i) for m in (2 * t + 2, 2 * t + 3) for i in range(m + 1) if (m, i) not in done])
        a = 2 * t + 3
        cand = [(m, i) for m in range(2 * t + 4, min(2 * t + 4 + NYS, NB)) for i in range(m + 1)
                if i <= a and m - i <= a and (m, i) not in done]
        nb, na = NBP.get(t, 0), NA.get(t + 1, 0)
        take((t, 'B'), cand[:nb])
        pend = cand[nb:nb + na]
        for c in pend:
            done.add(c)
    assert len(done) == NB * (NB + 1) // 2
    return plan


def _ln(x):
    m = jnp.mean(x, axis=-1, keepdims=True)
    xc = x - m
    v = jnp.mean(xc * xc, axis=-1, keepdims=True)
    return xc * jax.lax.rsqrt(v + EPS)


def _ln2(x):
    m = jnp.mean(x, axis=-1, keepdims=True)
    xc = x - m
    v = jnp.mean(xc * xc, axis=-1, keepdims=True)
    return xc * (0.5 * jax.lax.rsqrt(v + 4 * EPS))


def _gelu(x):
    c = np.float32(np.sqrt(2.0 / np.pi))
    inner = x * (c + (c * np.float32(0.044715)) * (x * x))
    return x + x * jnp.tanh(inner)


def _dot(a, b):
    return jnp.dot(a, b, preferred_element_type=F32)


class _NoScope:
    def __enter__(self): return self
    def __exit__(self, *a): return False


def _scope(name):
    return jax.named_scope(name) if SCOPES else _NoScope()


def kernel(q_hbm, k_hbm, v_hbm, shk_hbm, sk_hbm, sd_hbm, win_hbm, wsp_hbm, bsp_hbm, wout_hbm,
           f_hbm, g_hbm, zs_hbm, out_hbm,
           win_v, wsp_v, wout_v, z1_v, z2a_v, x_v3, y_v3, h_v, q_v3, bb_v,
           kv_v, sk_v, zt_v, shk_v, clk_v, shk_ref, sd_ref, bsp_ref, f_ref, g_ref, zs_ref,
           sem_in, sem_w, sem_s, sem_out, *bufs):
    sps, yss = bufs[:NT], bufs[NT:]
    x_v, y_v, q_v = x_v3.at[0], y_v3.at[0], q_v3.at[0]
    k_v = kv_v.at[:, 0:D]
    v_v = kv_v.at[:, D:2 * D]
    z2b_v = kv_v.at[:, 0:FH]
    u_v = sk_v.at[0:2 * TM, 0:FH]
    HS = [slice(n * TM, (n + 1) * TM) for n in range(4)]

    bi = lambda x: pltpu.bitcast(x, I32)
    hi = lambda w: pltpu.bitcast(w & np.int32(-65536), F32)
    lo = lambda w: pltpu.bitcast(w << 16, F32)
    pk = lambda a, b: bi(pltpu.pack_elementwise([a, b], packed_dtype=BF16))
    bc = lambda m: jnp.broadcast_to(m, (m.shape[0], 128))
    wide = lambda m, n: jnp.concatenate([m] * n, axis=1)
    rows8 = lambda x: [x[r:r + 8, c:c + 128] for r in range(0, x.shape[0], 8) for c in range(0, x.shape[1], 128)]
    half = lambda sl: slice(sl.start // 2, sl.stop // 2)
    cols = lambda x: [x[:, c:c + 128] for c in range(0, x.shape[1], 128)]

    WG = ((FH, FH + 2 * CN), (FH + 2 * CN, FH + 4 * CN), (FH + 4 * CN, F), (0, 5 * CN), (5 * CN, FH))
    wc = [pltpu.make_async_copy(win_hbm.at[:, a:b], win_v.at[:, a:b], sem_w.at[n]) for n, (a, b) in enumerate(WG)]
    def wsp_copy(n):
        r = pl.ds(pl.multiple_of(n * TM, TM), TM)
        return pltpu.make_async_copy(wsp_hbm.at[r], wsp_v.at[r], sem_w.at[7 + n])
    wout_copies = [pltpu.make_async_copy(wout_hbm.at[n * (FH // 2):(n + 1) * (FH // 2)],
                                         wout_v.at[n * (FH // 2):(n + 1) * (FH // 2)], sem_w.at[5 + n]) for n in range(2)]
    small = [pltpu.make_async_copy(a, b, sem_s.at[n]) for n, (a, b) in enumerate(
        [(zs_hbm, zs_ref), (f_hbm, f_ref), (shk_hbm, shk_ref), (sd_hbm, sd_ref), (bsp_hbm, bsp_ref), (g_hbm, g_ref)])]

    def tile_copies(t):
        r = pl.ds(t * TM, TM)
        return [pltpu.make_async_copy(k_hbm.at[0, r], k_v.at[r], sem_in.at[t, 0]),
                pltpu.make_async_copy(v_hbm.at[0, r], v_v.at[r], sem_in.at[t, 1]),
                pltpu.make_async_copy(sk_hbm.at[:, r], sk_v.at[:, r], sem_in.at[t, 2]),
                pltpu.make_async_copy(q_hbm.at[0, r], q_v.at[r], sem_in.at[t, 3])]
    inc = [tile_copies(t) for t in range(NT)]

    def start(cs):
        for c in cs:
            c.start()

    def wait(cs):
        for c in cs:
            c.wait()

    def a_layer(x, y, rows, hs):
        x1 = x + _ln(x) * y
        x_v[rows, :] = x1
        h_v[half(hs), :] = bi(_ln(x1).astype(BF16))

    def mm2(rows, hs, z2_src, act=False):
        bb = wide(bb_v[rows, :], CN // 128)
        for c in range(NC):
            cs = slice(c * CN, (c + 1) * CN)
            g = _dot(wsp_v[rows, :], pltpu.bitcast(z2_src[:, cs], BF16)) + bb
            z1 = z1_v[rows, cs]
            u_v[hs, cs] = ((_gelu(z1) if act else z1) * g).astype(BF16)

    def mm3(rows, hs):
        return x_v[rows, :] + _dot(u_v[hs, :], wout_v[...])

    with _scope("pro_init"):
        first = small[0:5] + inc[0][2:3]
        start(first)
        for sm, grp in zip(first, (inc[0][0:2] + small[5:], [inc[0][3]], inc[1][0:3], [wc[0]], [inc[1][3], wc[1]],
                                   [wc[2]])):
            sm.wait()
            start(grp)
    z0 = zs_ref[0]
    dz = [z0 * k for k in range(4)]
    zm = jnp.full((8, 128), z0, I32)
    with _scope("pro_bb"):
        shk_v[...] = shk_ref[...].astype(F32)
        bb_v[...] = jnp.transpose(jnp.broadcast_to(0.5 * bsp_ref[...].astype(F32).reshape(1, S), (128, S)))

    st = {"hprev": None, "clk": jax.lax.broadcasted_iota(I32, (8, 128), 1) & zm}
    qs = {}
    started = set()

    def lnk(h):
        h00 = pltpu.bitcast(bi(h[0:16, 0:128]) | st["clk"], BF16)
        return jnp.concatenate([jnp.concatenate([h00, h[0:16, 128:]], axis=1), h[16:]], axis=0)

    def lhs(hs):
        w = h_v[half(hs), :]
        w0 = jnp.concatenate([w[0:8, 0:128] | st["clk"], w[0:8, 128:]], axis=1)
        return pltpu.bitcast(jnp.concatenate([w0, w[8:]], axis=0), BF16)

    def rs(base, off, n):
        if isinstance(base, int):
            return slice(base + off, base + off + n)
        return pl.ds(pl.multiple_of(base + off, n), n)

    def z2_step(hs, zr, c):
        zt_v[0, zr, c * CN:(c + 1) * CN] = _gelu(_dot(lhs(hs), win_v[:, FH + c * CN:FH + (c + 1) * CN]))

    def z1_step(hs, rows, act, c):
        z = _dot(lhs(hs), win_v[:, c * CN:(c + 1) * CN])
        z1_v[rows, c * CN:(c + 1) * CN] = _gelu(z) if act else z

    def g_step(rows, us, c):
        cs = slice(c * CN, (c + 1) * CN)
        g = _dot(lnk(wsp_v[rows, :]), pltpu.bitcast(z2a_v[:, cs], BF16)) + wide(bb_v[rows, :], CN // 128)
        u_v[us, cs] = (_gelu(z1_v[rows, cs]) * g).astype(BF16)

    def o_step(rows, us, xt, link, c):
        cs = slice(c * CN, (c + 1) * CN)
        u = u_v[us, :]
        xt[0, 0:u.shape[0], cs] = x_v[rows, cs] + _dot(lnk(u) if link else u, wout_v[:, cs])

    def ssum(xs):
        s_ = xs[0]
        for v in xs[1:]:
            s_ = s_ + v
        return jnp.sum(s_, axis=-1, keepdims=True) * (1.0 / (128 * len(xs)))

    def st_mean(key, x):
        m = qs[key] = bc(ssum(cols(x)))
        return [bi(m)]

    def st_rstd(key, mkey, x, half=False):
        m = qs[mkey]
        xc = [v - m for v in cols(x)]
        r = jax.lax.rsqrt(ssum([v * v for v in xc]) + (4 * EPS if half else EPS))
        r = qs[key] = bc(0.5 * r if half else r)
        return [bi(r)]

    def st_out(dst, r0, gp, ld, w, mkey, rkey):
        g, p = gp // 2, gp % 2
        cs = slice(p * w // 2, (p + 1) * w // 2)
        x = ld(g, cs)
        n = x.shape[1] // 128
        m = jnp.concatenate([pltpu.bitcast(bi(qs[mkey, 2 * g + j]) | st["clk"], F32) for j in range(2)], axis=0)
        r = jnp.concatenate([qs[rkey, 2 * g + j] for j in range(2)], axis=0)
        o = ((x - wide(m, n)) * wide(r, n)).astype(BF16)
        if dst is h_v or dst is z2a_v:
            dst[half(rs(r0, 16 * g, 16)), cs] = bi(o)
        else:
            dst[rs(r0, 16 * g, 16), cs] = o
        return []

    def nrm_q(cx, g, stage):
        dst, base, z0r = cx
        if stage == 0:
            return st_mean(('nm', g), zt_v[dz[1], rs(z0r, 8 * g, 8), :])
        if stage == 1:
            return st_rstd(('nr', g), ('nm', g), zt_v[dz[2], rs(z0r, 8 * g, 8), :], True)
        return st_out(dst, base, g, lambda g, cs: zt_v[dz[3], rs(z0r, 16 * g, 16), cs], FH, 'nm', 'nr')

    def a_q(cx, g, stage):
        src, s0, base, xs, x0, h0 = cx
        r = rs(base, 8 * g, 8)
        if stage <= 2:
            x = src[dz[stage + 1], rs(s0, 8 * g, 8), :].astype(F32)
        if stage == 0:
            return st_mean(('am', g), x)
        if stage == 1:
            return st_rstd(('ar', g), ('am', g), x)
        if stage == 2:
            x1 = x + ((x - wide(qs['am', g], 8)) * wide(qs['ar', g], 8)) * y_v3[dz[1], r, :]
            x_v[r, :] = x1
            if xs is not x_v3:
                xs[0, rs(x0, 8 * g, 8), :] = x1
            return st_mean(('am', g), x1)
        if stage == 3:
            return st_rstd(('ar', g), ('am', g), xs[0, rs(x0, 8 * g, 8), :])
        return st_out(h_v, h0, g, lambda g, cs: xs[0, rs(x0, 16 * g, 16), cs], D, 'am', 'ar')

    def kv_q(m, c):
        cs = slice(c * 128, (c + 1) * 128)
        if m == 0:
            kw = jnp.concatenate([jnp.zeros((8, 128), I32), bi(k_v[0:B, cs])], axis=0)
        else:
            kw = bi(k_v[m * B - 16:(m + 1) * B, cs])
        k0 = kw[8:]
        k1 = pltpu.roll(kw, 1, axis=0)[8:]
        k2 = pltpu.roll(kw, 2, axis=0)[8:]
        w = [jnp.broadcast_to(shk_v[j:j + 1, cs], (8, 128)) for j in range(4)]
        vw = bi(v_v[m * B:(m + 1) * B, cs])
        out = []
        for n in range(8):
            r = slice(8 * n, 8 * n + 8)
            e0, o0, e1, o1, o2 = lo(k0[r]), hi(k0[r]), lo(k1[r]), hi(k1[r]), hi(k2[r])
            w0 = w[0] if (not out or m < 2) else pltpu.bitcast(bi(w[0]) | (out[-1] & zm), F32)
            se = ((e0 * w0 + o1 * w[1]) + e1 * w[2]) + o2 * w[3]
            so = ((o0 * w0 + e0 * w[1]) + o1 * w[2]) + e1 * w[3]
            out.append(pk(se * lo(vw[r]), so * hi(vw[r])))
        qs['kv', m, c] = jnp.concatenate(out, axis=0)
        return [out[-1]]

    def fwd_x(m):
        kvb = pltpu.bitcast(jnp.concatenate([qs.pop(('kv', m, c)) for c in range(8)], axis=1), BF16)
        xf = _dot(f_ref[...], kvb)
        sps[m // 2][m % 2, 0:B, OXC:OXC + D] = xf[0:B]
        sps[m // 2][m % 2, 0:B, OXS:OXS + D] = xf[B:2 * B]
        if m % 2:
            sps[m // 2][z0, 0:8, D:D + 128] = jnp.zeros((8, 128), F32)

    def fwd_h(m):
        hraw = jax.lax.dot_general(f_ref[...], sk_v[:, m * B:(m + 1) * B], (((1,), (1,)), ((), ())),
                                   preferred_element_type=F32)
        hprev = st["hprev"]
        hb = B // 2
        sp = sps[m // 2]
        if hprev is None:
            hraw = jnp.concatenate([hraw[0:B] + sd_ref[...].astype(F32).reshape(1, D), hraw[B:2 * B]], axis=0)
            sp[m % 2, 0:B, OHC:OHC + D] = hraw[0:B]
            sp[m % 2, 0:B, OHS:OHS + D] = hraw[B:2 * B]
        else:
            sp[m % 2, 0:hb, OHC:OHC + D] = hraw[0:hb] + hprev[B:B + hb]
            sp[m % 2, hb:B, OHC:OHC + D] = hraw[hb:B] - hprev[B + hb:2 * B]
            sp[m % 2, 0:hb, OHS:OHS + D] = hraw[B:B + hb] - hprev[0:hb]
            sp[m % 2, hb:B, OHS:OHS + D] = hraw[B + hb:2 * B] + hprev[hb:B]
        st["hprev"] = hraw

    def piece(m, iis, acc, final, R, W, p):
        nr = B // R
        r0 = (p % nr) * R
        c0 = (p // nr) * W
        ys = yss[m % NYS]
        yr = yi = None
        if acc:
            yr = ys[0, r0:r0 + R, c0:c0 + W]
            yi = ys[0, B + r0:B + r0 + R, c0:c0 + W]
        def ld(b, off):
            return sps[b // 2][b % 2, r0:r0 + R, off + c0:off + c0 + W]
        for i in iis:
            xr, xi, hr, hi_ = ld(i, OXC), ld(i, OXS), ld(m - i, OHC), ld(m - i, OHS)
            yr = (xr * hr if yr is None else yr + xr * hr) - xi * hi_
            yi = (xr * hi_ if yi is None else yi + xr * hi_) + xi * hr
        if final:
            r_ = qs['y', m, p] = pk(yr, yi)
            return rows8(r_)
        ys[0, r0:r0 + R, c0:c0 + W] = yr
        ys[0, B + r0:B + r0 + R, c0:c0 + W] = yi
        return rows8(bi(yr) | bi(yi))

    def pieces(jobs, final, R=PR, W=PW, interleave=False):
        out = []
        for m, iis in jobs:
            out.append([P(piece, m, iis, m in started, final, R, W, p) for p in range((B // R) * (D // W))])
            started.add(m)
        if interleave:
            return [(f_, len(j[1])) for fs in zip(*out) for f_, j in zip(fs, jobs)]
        return [(f_, len(j[1])) for fs, j in zip(out, jobs) for f_ in fs]

    def inv(t, R=PR, W=PW):
        nr = B // R
        for m in (2 * t, 2 * t + 1):
            ys = jnp.concatenate([jnp.concatenate([qs.pop(('y', m, c * nr + r)) for c in range(D // W)], axis=1)
                                  for r in range(nr)], axis=0)
            y_v[m * B:(m + 1) * B, :] = _dot(g_ref[...], pltpu.bitcast(ys, BF16))

    plan = _plan()

    def both(ws, ss, nm=[0]):
        def f_():
            nm[0] += 1
            with _scope("bar%d" % nm[0]):
                wait(ws)
            start(ss)
        return f_


    with _scope("pro_a"):
        fwd_h(0)
        fwd_h(1)
        both(inc[0][0:2], inc[2])()
        for m in (0, 1):
            for c in range(8):
                kv_q(m, c)
            fwd_x(m)
        both([inc[0][3]] + small[5:], [wc[3]])()
        for f_, _ in pieces([(0, [0]), (1, [0, 1])], True, 8, 512):
            f_()
        inv(0, 8, 512)
        for n in range(2):
            a_layer(q_v[n * B:(n + 1) * B, :].astype(F32), y_v3[z0, n * B:(n + 1) * B, :], slice(n * B, (n + 1) * B), rs(2 * TM, n * B, B))

    def paced(seq, barriers, fill, tstart=0):
        T = sum(c for _, c, _ in seq)
        tend = T - ENDM
        at, saved, ev, now = {}, {}, [], 0
        def run_mxu(fn, kind):
            cur = st["clk"]
            st["clk"] = saved[kind]
            fn()
            st["clk"] = cur
        def save_clk(kind):
            saved[kind] = st["clk"]
        prev_emit = 0
        for fn, c, kind in seq:
            at[kind] = now
            if kind in barriers:
                ev.append((prev_emit + 1, barriers[kind], None))
                at['b' + kind] = prev_emit + 2
            ev.append((max(now - MARGIN, 0), P(save_clk, kind), None))
            prev_emit = now + LATE * c // 1024
            ev.append((prev_emit, P(run_mxu, fn, kind), None))
            now += c
        def spread(fns, t0, t1, dl):
            t1 = min(t1, tend - dl * TICK)
            fns = [f_ if isinstance(f_, tuple) else (f_, 1) for f_ in fns]
            tot = sum(w for _, w in fns)
            acc = 0
            for fn, w in fns:
                ev.append((t0 + (t1 - t0) * acc / tot, fn, dl))
                acc += w
        def stages(fn, cx, stgs, ng, t0, t1):
            t1 = t1 - (len(stgs) + 1) * SG
            for j, stg in enumerate(stgs):
                last = stg == (2 if fn is nrm_q else 4)
                off = j * SG + (SG if last else 0)
                spread([P(fn, cx, g, stg) for g in range(ng)], t0 + off, t1 + off, LND)
        fill(at, tend, spread, stages)
        ev.sort(key=lambda e: e[0])
        ties, n = {}, 0
        for k in range(int(T / TICK) + 2):
            while n < len(ev) and ev[n][0] < (k + 1) * TICK:
                r = ev[n][1]()
                if ev[n][2] is not None:
                    ties.setdefault(k + ev[n][2], []).extend(r)
                n += 1
            c = st["clk"]
            tl = ties.pop(k + 1, None)
            if tl:
                while len(tl) > 1:
                    tl = [tl[j] | tl[j + 1] if j + 1 < len(tl) else tl[j] for j in range(0, len(tl), 2)]
                c = c | (tl[0] & zm)
            st["clk"] = pltpu.roll(c, 1, axis=1) if tstart <= (k + 1) * TICK <= tend else c
        assert n == len(ev) and not any(ties.values())

    extra = iter([(0, c) for c in range(NC)] + [(1, NC - 2), (1, NC - 1)])

    def norm0():
        z2a_v[half(HS[0]), :] = bi(_ln2(zt_v[z0]).astype(BF16))

    def region(t, order, barriers):
        conv = t + 1 < NT
        hs = HS[t % 2] if t > 1 else HS[2 + t]
        seq = []
        for kind in order.split():
            n = int(kind[1:] or 0)
            if kind[0] == 'h':
                seq.append((P(fwd_h, 2 * t + 2 + n), 512, kind))
            elif kind[0] == 'x':
                seq.append((P(fwd_x, 2 * t + 2 + n), 512, kind))
            elif kind[0] == 'i':
                seq.append((P(inv, t + 1), 1024, kind))
            elif kind[0] == 'e':
                te, c = next(extra)
                seq.append((P(z1_step, HS[2 + te], HS[te], False, c), 1024, kind))
            elif kind[0] == 'a':
                seq.append((lambda: a_layer(q_v[HS[1], :].astype(F32), y_v3[z0, HS[1], :], HS[1], HS[3]), 0, kind))
            elif kind[0] == 'n':
                seq.append((norm0, 0, kind))
            elif kind[0] == 'w':
                seq.append((lambda: None, n, kind))
            else:
                seq.append((P(z2_step, hs, HS[0], n) if n < NC else
                            P(z1_step, hs, rs(t * TM, 0, TM), False, n - NC), 1024, kind))
        def fill(at, tend, spread, stages):
            if t:
                stages(nrm_q, (z2a_v, t * TM, 0), (0, 1, 2), 32, at['s6'] + 1524, tend)
            if conv:
                t0 = at.get('bh0', 0)
                mid = (t0 + at['x1'] - 800) // 2
                spread([P(kv_q, 2 * t + 2, c) for c in range(8)], t0, min(mid, at['x0'] - 800), KVD)
                spread([P(kv_q, 2 * t + 3, c) for c in range(8)], min(mid, at['x0'] - 800), at['x1'] - 800, KVD)
                b1 = (t + 1) * TM
                cx = (q_v3, b1, b1, x_v3, b1, ((t + 1) % 2) * TM)
                if t:
                    stages(a_q, cx, (0, 1), 32, at['i'] - 3000, at['i'] + 1000)
                    stages(a_q, cx, (2, 3, 4), 32, at['i'] + 1500, tend)
                spread(pieces(plan[t, 'A'], False), 0, at['x1'] + 1000, HD)
                spread(pieces(plan[t, 'H'], True, interleave=True), at['x1'] + (1000 if t else 520), at['i'] - (700 if t else 300), HD)
                spread(pieces(plan[t, 'B'], False), at['i'] - 700, tend, HD)
        paced(seq, barriers, fill)

    for t in range(NT):
        barriers = {}
        order = ORD.get(t, ORD[2])
        if t == 0:
            both(inc[1][0:3], [wc[4]])()
            barriers['x1'] = both([wc[0]], [])
            barriers['i'] = both([inc[1][3], wc[1]], [])
            barriers['s4'] = both([wc[2]], [])
        elif t == 1:
            both(inc[2], inc[3])()
            barriers['x1'] = both([wc[3]], [])
        elif t + 1 < NT:
            wait(inc[t + 1] + ([wc[4]] if t == 2 else []) + ([wsp_copy(0)] if t == NT - 2 else []))
            start(inc[t + 2] + ([wsp_copy(0)] if t == NT - 3 else []) if t + 2 < NT else [wsp_copy(1)] + wout_copies)
        with _scope("p1_%d" % t):
            region(t, order, barriers)
    clk_v[...] = st["clk"]

    def rows1(i):
        return pl.ds(pl.multiple_of(i * TM, TM), TM)

    clk0 = jax.lax.broadcasted_iota(I32, (8, 128), 1) & zm
    NO = D // CN

    def p2(i, _):
        wsp_copy(i + 1).wait()

        @pl.when(i + 2 < NT)
        def _():
            wsp_copy(i + 2).start()

        st["clk"] = clk0
        base = pl.multiple_of(i * TM, TM)
        r = rows1(i)
        seq = [(P(o_step, r, HS[0], yss[0], False, c), FH, 'o%d' % c) for c in range(NO)]
        seq += [(P(g_step, rows1(i + 1), HS[0], c), S, 'g%d' % c) for c in range(NC)]
        seq += [(P(z2_step, HS[0], HS[0], c), D, 's%d' % c) for c in range(NC)]
        seq += [(P(z1_step, HS[0], r, False, c), D, 's%d' % (NC + c)) for c in range(NC)]
        def fill(at, tend, spread, stages):
            stages(a_q, (yss[0], 0, base, yss[1], 0, 0), (0, 1, 2, 3, 4), 32, at['g0'] + 1000, at['s0'] - 1500)
            stages(nrm_q, (z2b_v, base, 0), (0, 1, 2), 32, at['s7'] + 500, tend)
        paced(seq, {}, fill, FH * NO - 2 * MARGIN)
        clk_v[...] = st["clk"]
        return 0

    with _scope("p2"):
        mm2(slice(0, TM), HS[0], z2a_v, True)
        wait(wout_copies)
        with _scope("p2loop"):
            jax.lax.fori_loop(0, NT - 1, p2, 0)
        hm = TM // 2
        base = (NT - 1) * TM
        st["clk"] = clk0
        seq = []
        for n in range(2):
            seq += [(P(o_step, rs(base, n * hm, hm), rs(0, n * hm, hm), yss[2 * n], n > 0, c), FH // 2, 'o%d%d' % (n, c))
                    for c in range(NO)]
        for n in range(2):
            hs = rs(0, n * hm, hm)
            seq += [(P(z2_step, hs, hs, c), D // 2, 's%d%d' % (n, c)) for c in range(NC)]
            seq += [(P(z1_step, hs, rs(base, n * hm, hm), False, c), D // 2, 't%d%d' % (n, c)) for c in range(NC)]
        def fill(at, tend, spread, stages):
            stages(a_q, (yss[0], 0, base, yss[1], 0, 0), (0, 1, 2, 3, 4), 16, at['o10'] + 300, at['s00'] - 200)
            stages(a_q, (yss[2], 0, base + hm, yss[3], 0, hm), (0, 1, 2, 3, 4), 16, at['s00'] + 300, at['t00'] + 300)
            stages(nrm_q, (z2b_v, base, 0), (0, 1, 2), 16, at['t00'] + 400, at['s10'])
            stages(nrm_q, (z2b_v, base + hm, hm), (0, 1, 2), 16, at['t10'] + 400, tend)
        paced(seq, {}, fill, FH * NO // 2 - 2 * MARGIN)
        clk_v[...] = st["clk"]

    o_v = q_v
    def rows2(i):
        r0 = pl.multiple_of(i * (2 * TM), 2 * TM)
        return pl.ds(r0, TM), pl.ds(r0 + TM, TM)

    def out_copies(i):
        ra, rb = rows2(i)
        hd = D // 2
        return [pltpu.make_async_copy(o_v.at[ra], out_hbm.at[0, ra], sem_out.at[i, 0]),
                pltpu.make_async_copy(o_v.at[rb, 0:hd], out_hbm.at[0, rb, 0:hd], sem_out.at[i, 1]),
                pltpu.make_async_copy(o_v.at[rb, hd:D], out_hbm.at[0, rb, hd:D], sem_out.at[i, 2])]

    def p3(i, _):
        ra, rb = rows2(i)
        oc = out_copies(i)
        mm2(ra, HS[0], z2b_v, True)
        mm2(rb, HS[1], z2b_v, True)
        o_v[ra, :] = mm3(ra, HS[0]).astype(BF16)
        oc[0].start()
        for n in range(2):
            cs = slice(n * (D // 2), (n + 1) * (D // 2))
            o_v[rb, cs] = (x_v[rb, cs] + _dot(u_v[HS[1], :], wout_v[:, cs])).astype(BF16)
            oc[1 + n].start()
        return 0

    with _scope("p3"):
        jax.lax.fori_loop(0, NT // 2, p3, 0)
    with _scope("outwait"):
        for i in range(NT // 2):
            wait(out_copies(i))


@jax.jit
def pallas_interleave_layers__ssm_conv_h3__mixer_gmlp__prompt_kernel(A_q, A_k, A_v, A_shift_k, A_ssm_k, A_ssm_D, B_x, B_w_in, B_w_sp, B_b_sp, B_w_out):
    f, g = _dft_mats()
    any_ = pl.BlockSpec(memory_space=pl.ANY)
    return pl.pallas_call(
        kernel,
        out_shape=jax.ShapeDtypeStruct((1, S, D), BF16),
        in_specs=[any_] * 13,
        out_specs=any_,
        scratch_shapes=[
            pltpu.VMEM((D, F), BF16), pltpu.VMEM((S, S), BF16), pltpu.VMEM((FH, D), BF16),
            pltpu.VMEM((S, FH), F32), pltpu.VMEM((S // 2, FH), I32),
            pltpu.VMEM((1, S, D), F32), pltpu.VMEM((1, S, D), F32),
            pltpu.VMEM((2 * TM, D), I32), pltpu.VMEM((1, S, D), BF16),
            pltpu.VMEM((S, 128), F32),
            pltpu.VMEM((S, 2 * D), BF16), pltpu.VMEM((D, S), BF16),
            pltpu.VMEM((1, TM, FH), F32), pltpu.VMEM((4, D), F32), pltpu.VMEM((8, 128), I32),
            pltpu.VMEM((4, D), BF16), pltpu.VMEM((D,), BF16), pltpu.VMEM((S,), BF16),
            pltpu.VMEM((2 * B, B), BF16), pltpu.VMEM((B, 2 * B), BF16), pltpu.SMEM((1,), I32),
            pltpu.SemaphoreType.DMA((NT, 4)), pltpu.SemaphoreType.DMA((7 + NT,)), pltpu.SemaphoreType.DMA((6,)),
            pltpu.SemaphoreType.DMA((NT // 2, 3)),
        ] + [pltpu.VMEM((2, B, WSP), F32)] * NT + [pltpu.VMEM((1, 2 * B, D), F32)] * NYS,
        compiler_params=pltpu.CompilerParams(vmem_limit_bytes=127 * 1024 * 1024),
    )(A_q, A_k, A_v, A_shift_k.T, A_ssm_k, A_ssm_D, B_w_in, B_w_sp, B_b_sp, B_w_out,
      jnp.asarray(f, BF16), jnp.asarray(g, BF16), jnp.asarray(np.zeros((1,), np.int32)))
```
